```python
import jax
import jax.numpy as jnp

def _softmax(x, axis=-1):
    return jax.nn.softmax(x, axis=axis)
def _gelu(x):
    return jax.nn.gelu(x, approximate=True)
def _silu(x):
    return jax.nn.silu(x)
def _sigmoid(x):
    return jax.nn.sigmoid(x)
def _layernorm(x, axis=-1, eps=1e-5):
    m = jnp.mean(x, axis=axis, keepdims=True)
    v = jnp.var(x, axis=axis, keepdims=True)
    return (x - m) / jnp.sqrt(v + eps)
def _scatter_add(tgt, idx, src, axis=0):
    return tgt.at[idx].add(src)
def _segment_sum(src, seg, n):
    return jax.ops.segment_sum(src, seg, n)
class _Rng:
    def __init__(self, key):
        self._k = key
    def _next(self):
        self._k, sub = jax.random.split(self._k)
        return sub
    def normal(self, shape):
        return jax.random.normal(self._next(), shape, dtype=jnp.bfloat16)
    def randint(self, lo, hi, shape):
        return jax.random.randint(self._next(), shape, lo, hi, dtype=jnp.int32)
    def uniform(self, shape, lo=0.0, hi=1.0):
        return jax.random.uniform(self._next(), shape, jnp.bfloat16, lo, hi)
    def permutation(self, n):
        return jax.random.permutation(self._next(), n)


kernel_name = 'interleave_layers__sliding_block_cached__mixer_s_mlp__decode'

def setup_inputs():
    _rng = _Rng(jax.random.key(int.from_bytes(__import__("os").urandom(4), "little")))
    _w = (lambda a: (lambda t: t.astype(jnp.bfloat16) if jnp.issubdtype(t.dtype, jnp.floating) else t)(jnp.asarray(a)))
    def _A_setup():
        B, Sq, D = 1, 1, 640
        Hq, Hkv, Sk, Dh = 32, 32, 32768, 192
        assert Hq % Hkv == 0, (Hq, Hkv)
        return {
            "x": _w((lambda *s: _rng.normal(s) * 0.05)(B, Sq, D)),
            "k_cache": _w((lambda *s: _rng.normal(s) * 0.05)(B, Hkv, Sk, Dh)),
            "v_cache": _w((lambda *s: _rng.normal(s) * 0.05)(B, Hkv, Sk, Dh)),
            "wq": _w((lambda *s: _rng.normal(s) * 0.05)(D, Hq * Dh) * (D ** -0.5)),
            "wo": _w((lambda *s: _rng.normal(s) * 0.05)(Hq * Dh, D) * ((Hq * Dh) ** -0.5)),
        }
    _A_in = _A_setup()

    def _B_setup():
        B, S, D, F = 1, 1, 640, 1536
        return {
            "x":  _w((lambda *s: _rng.normal(s) * 0.05)(B, S, D)),
            "w1": _w((lambda *s: _rng.normal(s) * 0.05)(D, D) * (D ** -0.5)),
            "w2": _w((lambda *s: _rng.normal(s) * 0.05)(D, D) * (D ** -0.5)),
            "w3": _w((lambda *s: _rng.normal(s) * 0.05)(D, F) * (D ** -0.5)),
            "w4": _w((lambda *s: _rng.normal(s) * 0.05)(F, D) * (F ** -0.5)),
        }
    _B_in = _B_setup()

    return {
        "A_x": _A_in["x"],
        "A_k_cache": _A_in["k_cache"],
        "A_v_cache": _A_in["v_cache"],
        "A_wq": _A_in["wq"],
        "A_wo": _A_in["wo"],
        "B_x": _B_in["x"],
        "B_w1": _B_in["w1"],
        "B_w2": _B_in["w2"],
        "B_w3": _B_in["w3"],
        "B_w4": _B_in["w4"],
    }

def reference(A_x, A_k_cache, A_v_cache, A_wq, A_wo, B_x, B_w1, B_w2, B_w3, B_w4):
    def _A_ref(x, k_cache, v_cache, wq, wo):
        B, Sq, D = x.shape
        Hq, Dh = 32, 192
        Hkv, Sk = k_cache.shape[1], k_cache.shape[2]
        W = min(4096, max(256, Sk // 4))
        rep = Hq // Hkv
        q = (lambda x, *d: x.transpose(*d))((x @ wq).reshape(B, Sq, Hq, Dh), 0, 2, 1, 3)
        k = jnp.repeat(k_cache[:, :, Sk - W:, :], rep, axis=1)
        v = jnp.repeat(v_cache[:, :, Sk - W:, :], rep, axis=1)
        scores = jnp.einsum("bhqd,bhkd->bhqk", q, k) * (Dh ** -0.5)
        p = _softmax(scores, axis=-1)
        o = jnp.einsum("bhqk,bhkd->bhqd", p, v)
        return (lambda x, *d: x.transpose(*d))(o, 0, 2, 1, 3).reshape(B, Sq, Hq * Dh) @ wo

    def _B_ref(x, w1, w2, w3, w4):
        B, S, D = x.shape
        h = _gelu(_layernorm(x, axis=-1) @ w1)
        c = D // 4
        g0 = jnp.pad(h[:, :, 0*c:1*c], ((0, 0), (1, 0), (0, 0)))[:, :S, :]
        g1 = jnp.pad(h[:, :, 1*c:2*c], ((0, 0), (0, 1), (0, 0)))[:, 1:, :]
        g2 = jnp.pad(h[:, :, 2*c:3*c], ((0, 0), (2, 0), (0, 0)))[:, :S, :]
        g3 = jnp.pad(h[:, :, 3*c:   ], ((0, 0), (0, 2), (0, 0)))[:, 2:, :]
        hs = jnp.concatenate([g0, g1, g2, g3], axis=-1) @ w2
        x1 = x + hs
        h2 = _gelu(_layernorm(x1, axis=-1) @ w3) @ w4
        return x1 + h2

    x = A_x
    x = x + _A_ref(_layernorm(x, axis=-1), A_k_cache, A_v_cache, A_wq, A_wo)
    x = x + _B_ref(_layernorm(x, axis=-1), B_w1, B_w2, B_w3, B_w4)
    x = x + _A_ref(_layernorm(x, axis=-1), A_k_cache, A_v_cache, A_wq, A_wo)
    x = x + _B_ref(_layernorm(x, axis=-1), B_w1, B_w2, B_w3, B_w4)
    return x
```

```python
import functools

import jax
import jax.numpy as jnp
import jax.experimental.pallas as pl
import jax.experimental.pallas.tpu as pltpu

H = 32
DH = 192
D = 640
F = 1536
LANES = 128
NP = H // 2
EPS = 1e-5


def _ln(x):
    m = jnp.mean(x, axis=-1, keepdims=True)
    d = x - m
    v = jnp.mean(d * d, axis=-1, keepdims=True)
    return d / jnp.sqrt(v + EPS)


def _expand64(x, upper, lane):
    if upper:
        x = pltpu.roll(x, 64, 1)
    y = jnp.where((lane & 64) != 0, pltpu.roll(x, 32, 1), x)
    z = jnp.where((lane & 32) != 0, pltpu.roll(y, 16, 1), y)
    w = jnp.where((lane & 16) != 0, pltpu.roll(z, 8, 1), z)
    return jnp.where((lane & 8) != 0, pltpu.roll(w, 8, 1), w)


def _kernel(x_ref, k_hbm, v_hbm, wq_hbm, wo_hbm, w3_hbm, w4_hbm, o_ref,
            kb, vb, wqb, wob, w3b, w4b, p_scr, oacc, sems, *, w_rows, n_rows):
    k32 = k_hbm.bitcast(jnp.uint32)
    v32 = v_hbm.bitcast(jnp.uint32)
    r0 = n_rows - w_rows

    def cp_k(j):
        return pltpu.make_async_copy(
            k32.at[pl.ds(2 * j, 2), :, pl.ds(r0, w_rows), :], kb.at[pl.ds(2 * j, 2)], sems.at[j])

    def cp_v(j):
        return pltpu.make_async_copy(
            v32.at[pl.ds(2 * j, 2), :, pl.ds(r0, w_rows), :], vb.at[pl.ds(2 * j, 2)], sems.at[NP + j])

    def cp_wo(j):
        return pltpu.make_async_copy(
            wo_hbm.at[pl.ds(2 * DH * j, 2 * DH), :], wob.at[j], sems.at[2 * NP + j])

    def cp_wq(j):
        return pltpu.make_async_copy(
            wq_hbm.at[:, pl.ds(2 * DH * j, 2 * DH)], wqb.at[j], sems.at[3 * NP + j])

    cp_w3 = pltpu.make_async_copy(w3_hbm, w3b, sems.at[4 * NP])
    cp_w4 = pltpu.make_async_copy(w4_hbm, w4b, sems.at[4 * NP + 1])

    cp_wq(0).start()
    cp_k(0).start()
    for j in range(1, NP):
        cp_wq(j).start()
    cp_v(0).start()
    cp_wo(0).start()
    cp_k(1).start()
    cp_v(1).start()
    cp_wo(1).start()

    lane = jax.lax.broadcasted_iota(jnp.int32, (8, LANES), 1)
    sub = jax.lax.broadcasted_iota(jnp.int32, (8, LANES), 0)
    half = jnp.where((lane & 8) != 0, jnp.uint32(0xFFFF0000), jnp.uint32(0x0000FFFF))
    scale = DH ** -0.5

    def stage_a(j, xq):
        q = jnp.dot(xq, wqb[j], preferred_element_type=jnp.float32)
        qw = pltpu.bitcast(q.astype(jnp.bfloat16), jnp.uint32)
        ps = []
        for hh in range(2):
            bases = []
            for g in range(3):
                s = 3 * hh + g
                b = _expand64(qw[:, LANES * (s // 2):LANES * (s // 2 + 1)], s % 2 == 1, lane)
                bases.append(b & half)
            tiles = []
            for jj in range(8):
                for g in range(3):
                    t = jnp.where(sub == jj, bases[g], jnp.uint32(0))
                    tiles.append(pltpu.bitcast(t, jnp.bfloat16))
            lhs = jnp.concatenate(tiles, axis=1)
            sc = []
            for cc in range(2):
                ws = []
                for jj in range(8):
                    cpi = cc * 8 + jj
                    for g in range(3):
                        w = kb[2 * j + hh, pl.ds(8 * g, 8), pl.ds(8 * cpi, 8), :]
                        ws.append(pltpu.bitcast(w, jnp.bfloat16).reshape(128, LANES))
                wmat = jnp.concatenate(ws, axis=0)
                sc.append(jnp.dot(lhs, wmat, preferred_element_type=jnp.float32))
            s = jnp.concatenate(sc, axis=0) * scale
            m = jnp.max(jnp.max(s, axis=1, keepdims=True), axis=0, keepdims=True)
            e = jnp.exp(s - m)
            l = jnp.sum(jnp.sum(e, axis=1, keepdims=True), axis=0, keepdims=True)
            ps.append(e * (1.0 / l))
        return jnp.concatenate(ps, axis=0)

    def stage_b(j, p, out):
        p_scr[...] = p
        for hh in range(2):
            acc = [jnp.zeros((8, LANES), jnp.float32) for _ in range(24)]
            for cpi in range(16):
                p0 = jnp.broadcast_to(p_scr[pl.ds(32 * hh + 2 * cpi, 1), :], (8, LANES))
                p1 = jnp.broadcast_to(p_scr[pl.ds(32 * hh + 2 * cpi + 1, 1), :], (8, LANES))
                for r in range(24):
                    w = vb[2 * j + hh, r, pl.ds(8 * cpi, 8), :]
                    vf = pltpu.bitcast(w, jnp.bfloat16).astype(jnp.float32)
                    acc[r] = acc[r] + (vf[0:8] * p0 + vf[8:16] * p1)
            oacc[pl.ds(DH * hh, DH), :] = jnp.concatenate(acc, axis=0)
        ot = oacc[...].T
        fold = ot.reshape(8, 16, 2 * DH).sum(axis=0)
        return out + jnp.dot(fold.astype(jnp.bfloat16), wob[j], preferred_element_type=jnp.float32)

    def attention(x, first):
        xq = jnp.broadcast_to(_ln(x), (16, D)).astype(jnp.bfloat16)
        if first:
            cp_wq(0).wait()
            cp_k(0).wait()
        p = stage_a(0, xq)

        def body(j, carry):
            p, out = carry
            if first:
                cp_wq(j).wait()
                cp_k(j).wait()
                cp_v(j - 1).wait()
                cp_wo(j - 1).wait()

                @pl.when(j + 1 < NP)
                def _():
                    cp_k(j + 1).start()

                @pl.when(j + 1 == NP)
                def _():
                    cp_w3.start()
                    cp_w4.start()

                @pl.when(j < NP)
                def _():
                    pass
            out = stage_b(j - 1, p, out)
            p = stage_a(j, xq)
            if first:
                @pl.when(j + 1 < NP)
                def _():
                    cp_v(j + 1).start()
                    cp_wo(j + 1).start()
            return p, out

        p, out = jax.lax.fori_loop(1, NP, body, (p, jnp.zeros((16, D), jnp.float32)))
        if first:
            cp_v(NP - 1).wait()
            cp_wo(NP - 1).wait()
        out = stage_b(NP - 1, p, out)
        return x + jnp.sum(out, axis=0, keepdims=True)

    def mixer(x, first):
        y = _ln(x)
        z = jnp.broadcast_to(_ln(y), (16, D)).astype(jnp.bfloat16)
        if first:
            cp_w3.wait()
        h = jnp.dot(z, w3b[...], preferred_element_type=jnp.float32)
        h = jax.nn.gelu(h, approximate=True).astype(jnp.bfloat16)
        if first:
            cp_w4.wait()
        h2 = jnp.dot(h, w4b[...], preferred_element_type=jnp.float32)[0:1]
        return x + (y + h2)

    x = x_ref[...].astype(jnp.float32)
    x = attention(x, True)
    x = mixer(x, True)
    x = attention(x, False)
    x = mixer(x, False)
    o_ref[...] = x.astype(o_ref.dtype)


def _tile_view(c):
    _, h, s, dh = c.shape
    return (c.reshape(h, s // LANES, LANES, dh // 8, 8)
            .transpose(0, 3, 1, 4, 2)
            .reshape(h, dh // 8, s // LANES * 8, LANES))


@jax.jit
def pallas_interleave_layers__sliding_block_cached__mixer_s_mlp__decode_kernel(
    A_x: jax.Array,
    A_k_cache: jax.Array,
    A_v_cache: jax.Array,
    A_wq: jax.Array,
    A_wo: jax.Array,
    B_x: jax.Array,
    B_w1: jax.Array,
    B_w2: jax.Array,
    B_w3: jax.Array,
    B_w4: jax.Array,
):
    del B_x, B_w1, B_w2
    s = A_k_cache.shape[2]
    w = min(4096, max(256, s // 4))
    w_rows = w // LANES * 4
    n_rows = s // LANES * 4
    kk = _tile_view(A_k_cache)
    vv = _tile_view(A_v_cache)
    any_spec = pl.BlockSpec(memory_space=pl.ANY)
    out = pl.pallas_call(
        functools.partial(_kernel, w_rows=w_rows, n_rows=n_rows),
        out_shape=jax.ShapeDtypeStruct((1, D), A_x.dtype),
        in_specs=[pl.BlockSpec(memory_space=pltpu.VMEM)] + [any_spec] * 6,
        out_specs=pl.BlockSpec(memory_space=pltpu.VMEM),
        scratch_shapes=[
            pltpu.VMEM((H, 24, w_rows, LANES), jnp.uint32),
            pltpu.VMEM((H, 24, w_rows, LANES), jnp.uint32),
            pltpu.VMEM((NP, D, 2 * DH), jnp.bfloat16),
            pltpu.VMEM((NP, 2 * DH, D), jnp.bfloat16),
            pltpu.VMEM((D, F), jnp.bfloat16),
            pltpu.VMEM((F, D), jnp.bfloat16),
            pltpu.VMEM((64, LANES), jnp.float32),
            pltpu.VMEM((2 * DH, LANES), jnp.float32),
            pltpu.SemaphoreType.DMA((4 * NP + 2,)),
        ],
        compiler_params=pltpu.CompilerParams(vmem_limit_bytes=127 * 1024 * 1024),
    )(A_x.reshape(1, D), kk, vv, A_wq, A_wo, B_w3, B_w4)
    return out.reshape(A_x.shape)
```

```python
import functools

import jax
import jax.numpy as jnp
import jax.experimental.pallas as pl
import jax.experimental.pallas.tpu as pltpu

H = 32
DH = 192
D = 640
F = 1536
LANES = 128
NP = H // 2
EPS = 1e-5


def _ln(x):
    m = jnp.mean(x, axis=-1, keepdims=True)
    d = x - m
    v = jnp.mean(d * d, axis=-1, keepdims=True)
    return d / jnp.sqrt(v + EPS)


def _expand64(x, upper, lane):
    if upper:
        x = pltpu.roll(x, 64, 1)
    y = jnp.where((lane & 64) != 0, pltpu.roll(x, 32, 1), x)
    z = jnp.where((lane & 32) != 0, pltpu.roll(y, 16, 1), y)
    w = jnp.where((lane & 16) != 0, pltpu.roll(z, 8, 1), z)
    return jnp.where((lane & 8) != 0, pltpu.roll(w, 8, 1), w)


R_O, R_S, R_B, R_Q, R_OUT, R_P, R_END = 0, 768, 896, 992, 1016, 1096, 1224
NC = 8


def _f2u(x):
    return pltpu.bitcast(x, jnp.uint32)


def _u2f(x):
    return pltpu.bitcast(x, jnp.float32)


class _Attn:
    def __init__(self, kb, vb, wqb, wob, buf, zs):
        self.kb, self.vb, self.wqb, self.wob, self.buf = kb, vb, wqb, wob, buf
        self.z = [pl.multiple_of(zs[k], 8) for k in range(8)]
        self.lane = jax.lax.broadcasted_iota(jnp.int32, (8, LANES), 1)
        self.sub = jax.lax.broadcasted_iota(jnp.int32, (8, LANES), 0)
        self.half = jnp.where((self.lane & 8) != 0, jnp.uint32(0xFFFF0000), jnp.uint32(0x0000FFFF))

    def zero_out(self):
        self.buf[pl.ds(self.z[0] + R_OUT, 80), :] = jnp.zeros((80, LANES), jnp.float32)

    def read_out(self):
        o = jnp.concatenate(
            [self.buf[pl.ds(self.z[0] + R_OUT + 16 * v, 16), :] for v in range(5)], axis=1)
        return jnp.sum(o, axis=0, keepdims=True)

    def step(self, t, xq, *, q=True, qk=True, sm=True, pv=True, wo=True, guard=None, cfg=None):
        cfg = cfg or {}
        buf, z, lane, sub, half = self.buf, self.z, self.lane, self.sub, self.half
        kb, vb, wqb, wob = self.kb, self.vb, self.wqb, self.wob
        par = t & 1
        npar = 1 - par
        zq = z[0] + R_Q
        zb_w = z[1] + R_B + par * 48
        zb_r = z[1] + R_B + npar * 48
        zs_w = z[2] + R_S + par * 64
        zs_r = z[3] + R_S + npar * 64
        zp_w = z[4] + R_P + par * 64
        zp_r = z[5] + R_P + npar * 64
        zo_w = z[6] + R_O + par * 384
        zo_r = z[7] + R_O + npar * 384
        zout = z[0] + R_OUT
        scale = DH ** -0.5
        tmp = {}

        def q_mm(v):
            r = jnp.dot(xq, wqb[t + 1, :, pl.ds(LANES * v, LANES)], preferred_element_type=jnp.float32)
            buf[pl.ds(zq + 8 * v, 8), :] = _u2f(pltpu.bitcast(r.astype(jnp.bfloat16), jnp.uint32))

        def q_exp_load():
            xs = [_f2u(buf[pl.ds(zq + 8 * v, 8), :]) for v in range(3)]
            tmp['b'] = [_expand64(xs[s // 2], s % 2 == 1, lane) & half for s in range(6)]

        def q_exp_store():
            for s in range(6):
                buf[pl.ds(zb_w + 8 * s, 8), :] = _u2f(tmp['b'][s])

        def b_load():
            tmp['bases'] = [_f2u(buf[pl.ds(zb_r + 8 * s, 8), :]) for s in range(6)]

        def qk_unit(hh, cc, jj):
            d = None
            for g in range(3):
                lhs = pltpu.bitcast(jnp.where(sub == jj, tmp['bases'][3 * hh + g], jnp.uint32(0)), jnp.bfloat16)
                w = kb[2 * t + hh, pl.ds(8 * g, 8), pl.ds(8 * (cc * 8 + jj), 8), :]
                w = pltpu.bitcast(w, jnp.bfloat16).reshape(128, LANES)
                dd = jnp.dot(lhs, w, preferred_element_type=jnp.float32)
                d = dd if d is None else d + dd
            if jj > 0:
                d = tmp['sacc'] + d
            tmp['sacc'] = d
            buf[pl.ds(zs_w + 32 * hh + 16 * cc, 16), :] = d

        def sm_load(hh):
            s = buf[pl.ds(zs_r + 32 * hh, 32), :] * scale
            m = jnp.max(jnp.max(s, axis=1, keepdims=True), axis=0, keepdims=True)
            e = jnp.exp(s - m)
            l = jnp.sum(jnp.sum(e, axis=1, keepdims=True), axis=0, keepdims=True)
            tmp['p', hh] = e * (1.0 / l)

        def sm_store(hh):
            buf[pl.ds(zp_w + 32 * hh, 32), :] = tmp['p', hh]

        def wo_row(k):
            tmp['orow', k] = buf[pl.ds(zo_r + 8 * k, 8), :]

        def wo_fold():
            ot = jnp.concatenate([tmp['orow', k] for k in range(48)], axis=0).T
            tmp['fold'] = ot.reshape(8, 16, 2 * DH).sum(axis=0).astype(jnp.bfloat16)

        def out_load(v):
            tmp['out', v] = buf[pl.ds(zout + 16 * v, 16), :]

        def wo_mm(v):
            r = jnp.dot(tmp['fold'], wob[t - 3, :, pl.ds(LANES * v, LANES)], preferred_element_type=jnp.float32)
            buf[pl.ds(zout + 16 * v, 16), :] = tmp['out', v] + r

        def p_load(hh, c0):
            tmp['pc', hh, c0] = [jnp.broadcast_to(buf[pl.ds(zp_r + 32 * hh + c, 1), :], (8, LANES))
                                 for c in range(2 * c0, 2 * (c0 + NC))]

        def acc_load(hh, r, c0):
            tmp['oacc', hh, r, c0] = buf[pl.ds(zo_w + DH * hh + 8 * r, 8), :]

        def pv_unit(hh, r, c0):
            acc = None
            pcs = tmp['pc', hh, c0]
            for k in range(NC):
                w = vb[2 * (t - 2) + hh, r, pl.ds(8 * (c0 + k), 8), :]
                vf = pltpu.bitcast(w, jnp.bfloat16).astype(jnp.float32)
                u = vf[0:8] * pcs[2 * k] + vf[8:16] * pcs[2 * k + 1]
                acc = u if acc is None else acc + u
            if c0 > 0:
                acc = tmp['oacc', hh, r, c0] + acc
            buf[pl.ds(zo_w + DH * hh + 8 * r, 8), :] = acc

        fn = dict(qmm=q_mm, qexpl=q_exp_load, qexps=q_exp_store, bl=b_load, qk=qk_unit,
                  sml=sm_load, sms=sm_store, worow=wo_row, wof=wo_fold, ol=out_load, wo=wo_mm,
                  pl=p_load, al=acc_load, pv=pv_unit)
        stage_of = dict(qmm='q', qexpl='q', qexps='q', bl='qk', qk='qk', sml='sm', sms='sm', worow='wo',
                        wof='wo', ol='wo', wo='wo', pl='pv', al='pv', pv='pv')

        start = cfg.get('start', 0.12)
        span = cfg.get('span', 0.9)
        pos = []
        if pv:
            blocks = [(hh, c0) for hh in range(2) for c0 in range(0, 16, NC)]
            units = [('pv', hh, r, c0) for (hh, c0) in blocks for r in range(24)]
            n = len(units)
            for i, it in enumerate(units):
                pos.append(((i + 0.5) / n, it))
                if it[3] > 0:
                    pos.append(((i + 0.5 - cfg.get('aahead', 4)) / n - 1e-7, ('al',) + it[1:]))
            for b, (hh, c0) in enumerate(blocks):
                pos.append((b / len(blocks) - cfg.get('pahead', 0.02) if b else -0.9, ('pl', hh, c0)))
        qk_items = [(('qk', hh, cc, jj), 24) for hh in range(2) for cc in range(2) for jj in range(8)]
        q_items = [(('qmm', v), 40) for v in range(3)]
        wo_items = [(('wo', v), 24) for v in range(5)]
        qa, wa = cfg.get('q_at', 0), cfg.get('wo_at', 12)
        mx = qk_items[:qa] + q_items + qk_items[qa:wa] + wo_items + qk_items[wa:]
        tot = 1008.0
        acc = 0
        for it, w in mx:
            acc += w
            p_ = start + (span - start) * acc / tot
            pos.append((p_, it))
            if it[0] == 'wo':
                pos.append((p_ - cfg.get('oahead', 0.03), ('ol', it[1])))
            if it == ('qmm', 2):
                pos.append((p_ + 1e-6, ('qexpl',)))
        if q:
            pos.append((cfg.get('qexp', 0.99), ('qexps',)))
        if qk:
            pos.append((-1.0, ('bl',)))
        if sm:
            pos.append((-0.8, ('sml', 0)))
            pos.append((-0.7, ('sml', 1)))
            pos.append((cfg.get('sms', 0.6), ('sms', 0)))
            pos.append((cfg.get('sms', 0.6) + 0.01, ('sms', 1)))
        if wo:
            rows = [16 * b + r for r in range(16) for b in range(3)]
            wl0, wl1 = cfg.get('wl0', 0.0), cfg.get('wl1', 0.2)
            for i, k in enumerate(rows):
                pos.append((wl0 + (wl1 - wl0) * i / 48, ('worow', k)))
            pos.append((wl1 + 1e-4, ('wof',)))
        on = dict(q=q, qk=qk, sm=sm, pv=pv, wo=wo)
        pos = [e for e in pos if on[stage_of[e[1][0]]]]
        pos.sort(key=lambda e: e[0])
        if guard is None:
            for _, it in pos:
                fn[it[0]](*it[1:])
        else:
            for stage in ('q', 'qk', 'sm', 'pv', 'wo'):
                items = [it for _, it in pos if stage_of[it[0]] == stage]

                def run(items=items):
                    for it in items:
                        fn[it[0]](*it[1:])
                guard(stage, run)


def _kernel(x_ref, zs, k_hbm, v_hbm, wq_hbm, wo_hbm, w3_hbm, w4_hbm, o_ref,
            kb, vb, wqb, wob, w3b, w4b, buf, sems, *, w_rows, n_rows):
    k32 = k_hbm.bitcast(jnp.uint32)
    v32 = v_hbm.bitcast(jnp.uint32)
    r0 = n_rows - w_rows

    def cp_k(j):
        return pltpu.make_async_copy(
            k32.at[pl.ds(2 * j, 2), :, pl.ds(r0, w_rows), :], kb.at[pl.ds(2 * j, 2)], sems.at[j])

    def cp_v(j):
        return pltpu.make_async_copy(
            v32.at[pl.ds(2 * j, 2), :, pl.ds(r0, w_rows), :], vb.at[pl.ds(2 * j, 2)], sems.at[NP + j])

    def cp_wo(j):
        return pltpu.make_async_copy(
            wo_hbm.at[pl.ds(2 * DH * j, 2 * DH), :], wob.at[j], sems.at[2 * NP + j])

    def cp_wq(j):
        return pltpu.make_async_copy(
            wq_hbm.at[:, pl.ds(2 * DH * j, 2 * DH)], wqb.at[j], sems.at[3 * NP + j])

    cp_w3 = pltpu.make_async_copy(w3_hbm, w3b, sems.at[4 * NP])
    cp_w4 = pltpu.make_async_copy(w4_hbm, w4b, sems.at[4 * NP + 1])

    def valid(j):
        return jnp.logical_and(j >= 0, j < NP)

    def clamp(j):
        return jnp.clip(j, 0, NP - 1)

    def start_group(t):
        for cp, j in ((cp_wq, t + 1), (cp_k, t), (cp_v, t - 2), (cp_wo, t - 3)):
            if isinstance(j, int):
                if 0 <= j < NP:
                    cp(j).start()
            else:
                @pl.when(valid(j))
                def _(cp=cp, j=j):
                    cp(clamp(j)).start()

    def wait_group(t):
        for cp, j in ((cp_wq, t + 1), (cp_k, t), (cp_v, t - 2), (cp_wo, t - 3)):
            @pl.when(valid(j))
            def _(cp=cp, j=j):
                cp(clamp(j)).wait()

    for t in (-1, 0, 1):
        start_group(t)

    att = _Attn(kb, vb, wqb, wob, buf, zs)

    def attention_streaming(x):
        xq = jnp.broadcast_to(_ln(x), (16, D)).astype(jnp.bfloat16)
        att.zero_out()

        def body(t, carry):
            wait_group(t)
            start_group(t + 3)

            @pl.when(t == NP - 1)
            def _():
                cp_w3.start()
                cp_w4.start()

            first = dict(q=-1, qk=0, sm=1, pv=2, wo=3)

            def guard(stage, run):
                pl.when(jnp.logical_and(t >= first[stage], t < first[stage] + NP))(run)
            att.step(t, xq, guard=guard)
            return carry
        jax.lax.fori_loop(-1, NP + 3, body, 0)
        return x + att.read_out()

    def attention_resident(x):
        xq = jnp.broadcast_to(_ln(x), (16, D)).astype(jnp.bfloat16)
        att.zero_out()
        att.step(-1, xq, qk=False, sm=False, pv=False, wo=False)
        att.step(0, xq, sm=False, pv=False, wo=False)
        att.step(1, xq, pv=False, wo=False)
        att.step(2, xq, wo=False)

        def body(t, carry):
            att.step(t, xq)
            return carry
        jax.lax.fori_loop(3, NP - 1, body, 0)
        att.step(NP - 1, xq, q=False)
        att.step(NP, xq, q=False, qk=False)
        att.step(NP + 1, xq, q=False, qk=False, sm=False)
        att.step(NP + 2, xq, q=False, qk=False, sm=False, pv=False)
        return x + att.read_out()

    def mixer(x, first):
        y = _ln(x)
        z = jnp.broadcast_to(_ln(y), (16, D)).astype(jnp.bfloat16)
        if first:
            cp_w3.wait()
        h = jnp.dot(z, w3b[...], preferred_element_type=jnp.float32)
        h = jax.nn.gelu(h, approximate=True).astype(jnp.bfloat16)
        if first:
            cp_w4.wait()
        h2 = jnp.dot(h, w4b[...], preferred_element_type=jnp.float32)[0:1]
        return x + (y + h2)

    x = x_ref[...].astype(jnp.float32)
    x = attention_streaming(x)
    x = mixer(x, True)
    x = attention_resident(x)
    x = mixer(x, False)
    o_ref[...] = x.astype(o_ref.dtype)


def _tile_view(c):
    _, h, s, dh = c.shape
    return (c.reshape(h, s // LANES, LANES, dh // 8, 8)
            .transpose(0, 3, 1, 4, 2)
            .reshape(h, dh // 8, s // LANES * 8, LANES))


@jax.jit
def pallas_interleave_layers__sliding_block_cached__mixer_s_mlp__decode_kernel(
    A_x: jax.Array,
    A_k_cache: jax.Array,
    A_v_cache: jax.Array,
    A_wq: jax.Array,
    A_wo: jax.Array,
    B_x: jax.Array,
    B_w1: jax.Array,
    B_w2: jax.Array,
    B_w3: jax.Array,
    B_w4: jax.Array,
):
    del B_x, B_w1, B_w2
    s = A_k_cache.shape[2]
    w = min(4096, max(256, s // 4))
    w_rows = w // LANES * 4
    n_rows = s // LANES * 4
    kk = _tile_view(A_k_cache)
    vv = _tile_view(A_v_cache)
    any_spec = pl.BlockSpec(memory_space=pl.ANY)
    out = pl.pallas_call(
        functools.partial(_kernel, w_rows=w_rows, n_rows=n_rows),
        out_shape=jax.ShapeDtypeStruct((1, D), A_x.dtype),
        in_specs=[pl.BlockSpec(memory_space=pltpu.VMEM), pl.BlockSpec(memory_space=pltpu.SMEM)] + [any_spec] * 6,
        out_specs=pl.BlockSpec(memory_space=pltpu.VMEM),
        scratch_shapes=[
            pltpu.VMEM((H, 24, w_rows, LANES), jnp.uint32),
            pltpu.VMEM((H, 24, w_rows, LANES), jnp.uint32),
            pltpu.VMEM((NP, D, 2 * DH), jnp.bfloat16),
            pltpu.VMEM((NP, 2 * DH, D), jnp.bfloat16),
            pltpu.VMEM((D, F), jnp.bfloat16),
            pltpu.VMEM((F, D), jnp.bfloat16),
            pltpu.VMEM((R_END, LANES), jnp.float32),
            pltpu.SemaphoreType.DMA((4 * NP + 2,)),
        ],
        compiler_params=pltpu.CompilerParams(vmem_limit_bytes=127 * 1024 * 1024),
    )(A_x.reshape(1, D), jnp.zeros((8,), jnp.int32), kk, vv, A_wq, A_wo, B_w3, B_w4)
    return out.reshape(A_x.shape)
```

```python
import functools

import jax
import jax.numpy as jnp
import jax.experimental.pallas as pl
import jax.experimental.pallas.tpu as pltpu

H = 32
DH = 192
D = 640
F = 1536
LANES = 128
NP = H // 2
EPS = 1e-5


def _ln(x):
    m = jnp.mean(x, axis=-1, keepdims=True)
    d = x - m
    v = jnp.mean(d * d, axis=-1, keepdims=True)
    return d * jax.lax.rsqrt(v + EPS)


def _ln_centred(y):
    m = jnp.mean(y, axis=-1, keepdims=True)
    v = jnp.mean(y * y, axis=-1, keepdims=True) - m * m
    return (y - m) * jax.lax.rsqrt(v + EPS)


R_O, R_S, R_B, R_Q, R_OUT, R_P, R_END = 0, 768, 896, 992, 1016, 1096, 1224
W4_CHUNKS = 4
CFG = dict(q_at=2, e_at=10, wo_at=20, start=0.16, span=0.9, start2=0.0, span2=0.81, bln=0.7,
           sms=0.9, wl0=0.0, wl1=0.2, aahead=8, pahead=0.01, nc=16, qexp=0.8)


def _f2u(x):
    return pltpu.bitcast(x, jnp.uint32)


def _u2f(x):
    return pltpu.bitcast(x, jnp.float32)


class _Attn:
    def __init__(self, kb, vb, wqb, wob, buf, zs, eb, xb):
        self.kb, self.vb, self.wqb, self.wob, self.buf = kb, vb, wqb, wob, buf
        self.eb, self.xb = eb, xb
        self.z = [pl.multiple_of(zs[k], 8) for k in range(8)]
        self.lane = jax.lax.broadcasted_iota(jnp.int32, (8, LANES), 1)
        self.sub = jax.lax.broadcasted_iota(jnp.int32, (8, LANES), 0)
        self.half = jnp.where((self.lane & 8) != 0, jnp.uint32(0xFFFF0000), jnp.uint32(0x0000FFFF))

    def init_expander(self):
        src = jax.lax.broadcasted_iota(jnp.int32, (LANES, LANES), 0)
        dst = jax.lax.broadcasted_iota(jnp.int32, (LANES, LANES), 1)
        for h in range(2):
            e = jnp.where(src == 64 * h + 8 * (dst >> 4) + (dst & 7), 1.0, 0.0).astype(jnp.bfloat16)
            self.eb[h] = pltpu.bitcast(e, jnp.uint32)

    def expand(self, rows):
        lhs = jnp.concatenate([rows, rows], axis=0).astype(jnp.bfloat16)
        outs = []
        for h in range(2):
            e = pltpu.bitcast(self.eb[h], jnp.bfloat16)
            ex = jnp.dot(lhs, e, preferred_element_type=jnp.float32)[0:8]
            b = _f2u(ex)
            outs.append((b | (b >> 16)) & self.half)
        return outs

    def set_x(self, x):
        xn = _ln(x).astype(jnp.bfloat16).astype(jnp.float32)
        rows = jnp.zeros((8, LANES), jnp.float32)
        for v in range(D // LANES):
            rows = jnp.where(self.sub == v, jnp.broadcast_to(xn[:, LANES * v:LANES * (v + 1)], (8, LANES)), rows)
        ex = self.expand(rows)
        for g in range(10):
            self.xb[g] = jnp.broadcast_to(ex[g % 2][g // 2:g // 2 + 1, :], (8, LANES))

    def zero_out(self):
        self.buf[pl.ds(self.z[0] + R_OUT, 80), :] = jnp.zeros((80, LANES), jnp.float32)

    def read_out(self):
        o = jnp.concatenate(
            [self.buf[pl.ds(self.z[0] + R_OUT + 16 * v, 16), :] for v in range(5)], axis=1)
        return jnp.sum(o, axis=0, keepdims=True)

    def step(self, t, *, q=True, qk=True, sm=True, pv=True, wo=True, guard=None, cfg=None,
             clamp_idx=False, grp=None, bases=None, next_bases=False):
        cfg = cfg or CFG
        buf, z, lane, sub, half = self.buf, self.z, self.lane, self.sub, self.half
        kb, vb, wqb, wob = self.kb, self.vb, self.wqb, self.wob
        par = t & 1 if grp is None else grp[1]
        npar = 1 - par
        zq = z[0] + R_Q
        bpar = par if grp is None else grp[0] & 1
        zb_w = z[1] + R_B + bpar * 16
        zb_r = z[1] + R_B + (1 - bpar) * 16
        zs_w = z[2] + R_S + par * 64
        zs_r = z[3] + R_S + npar * 64
        zp_w = z[4] + R_P + par * 64
        zp_r = z[5] + R_P + npar * 64
        zo_w = z[6] + R_O + par * 384
        zo_r = z[7] + R_O + npar * 384
        zout = z[0] + R_OUT
        scale = DH ** -0.5
        tmp = {}
        NC = cfg.get('nc', 8)
        if clamp_idx:
            jq, jk = jnp.minimum(t + 1, NP - 1), jnp.minimum(t, NP - 1)
            jv, jo = t - 2, jnp.maximum(t - 3, 0)
        else:
            jq, jk, jv, jo = t + 1, t, t - 2, t - 3

        def q_mm(g):
            xbase = self.xb[g]
            d = None
            if grp is None:
                c0, na = 3 * jq >> 1, 2
            else:
                gq = grp[0] + 1
                c0, na = 3 * (jnp.minimum(gq, NP // 2 - 1) if clamp_idx else gq), 3
            for a in range(na):
                lhs = pltpu.bitcast(jnp.where(sub == a, xbase, jnp.uint32(0)), jnp.bfloat16)
                w = wqb[pl.ds(8 * g, 8), pl.ds(pl.multiple_of(8 * (c0 + a), 8), 8), :]
                w = pltpu.bitcast(w, jnp.bfloat16).reshape(128, LANES)
                dd = jnp.dot(lhs, w, preferred_element_type=jnp.float32)[0:8]
                d = dd if d is None else d + dd
            if g > 0:
                d = (tmp['q'] if 'q' in tmp else buf[pl.ds(zq, 8), :]) + d
            tmp['q'] = d
            buf[pl.ds(zq, 8), :] = d

        def q_exp_load():
            tmp['b'] = self.expand(buf[pl.ds(zq, 8), :].astype(jnp.bfloat16).astype(jnp.float32))

        def q_exp_store():
            for h in range(2):
                buf[pl.ds(zb_w + 8 * h, 8), :] = _u2f(tmp['b'][h])

        def load_bases(odd):
            return [jnp.broadcast_to(_f2u(buf[pl.ds(zb_r + 8 * (s % 2) + odd + s // 2, 1), :]), (8, LANES))
                    for s in range(6)]

        def b_load():
            if bases is not None:
                tmp['bases'] = bases
            else:
                tmp['bases'] = load_bases(jk & 1 if grp is None else 3 * grp[1])

        def b_load_next():
            tmp['nb'] = load_bases(3)

        def qk_unit(hh, cc, jj):
            d = None
            for g in range(3):
                lhs = pltpu.bitcast(jnp.where(sub == jj, tmp['bases'][3 * hh + g], jnp.uint32(0)), jnp.bfloat16)
                w = kb[2 * jk + hh, pl.ds(8 * g, 8), pl.ds(8 * (cc * 8 + jj), 8), :]
                w = pltpu.bitcast(w, jnp.bfloat16).reshape(128, LANES)
                dd = jnp.dot(lhs, w, preferred_element_type=jnp.float32)
                d = dd if d is None else d + dd
            if jj > 0:
                d = tmp['sacc'] + d
            tmp['sacc'] = d
            buf[pl.ds(zs_w + 32 * hh + 16 * cc, 16), :] = d

        def sm_load(hh):
            s = buf[pl.ds(zs_r + 32 * hh, 32), :] * scale
            m = jnp.max(jnp.max(s, axis=1, keepdims=True), axis=0, keepdims=True)
            e = jnp.exp(s - m)
            l = jnp.sum(jnp.sum(e, axis=1, keepdims=True), axis=0, keepdims=True)
            tmp['p', hh] = e * (1.0 / l)

        def sm_store(hh):
            buf[pl.ds(zp_w + 32 * hh, 32), :] = tmp['p', hh]

        def wo_row(k):
            tmp['orow', k] = buf[pl.ds(zo_r + 8 * k, 8), :]

        def wo_fold():
            ot = jnp.concatenate([tmp['orow', k] for k in range(48)], axis=0).T
            tmp['fold'] = ot.reshape(8, 16, 2 * DH).sum(axis=0).astype(jnp.bfloat16)

        def out_load(v):
            tmp['out', v] = buf[pl.ds(zout + 16 * v, 16), :]

        def wo_mm(v):
            w = pltpu.bitcast(wob[jo, v], jnp.bfloat16)
            r = jnp.dot(tmp['fold'], w, preferred_element_type=jnp.float32)
            if clamp_idx:
                r = jnp.where(t >= 3, r, 0.0)
            buf[pl.ds(zout + 16 * v, 16), :] = tmp['out', v] + r

        def p_load(hh, c0):
            tmp['pc', hh, c0] = [jnp.broadcast_to(buf[pl.ds(zp_r + 32 * hh + c, 1), :], (8, LANES))
                                 for c in range(2 * c0, 2 * (c0 + NC))]

        def acc_load(hh, r, c0):
            tmp['oacc', hh, r, c0] = buf[pl.ds(zo_w + DH * hh + 8 * r, 8), :]

        def pv_unit(hh, r, c0):
            acc = None
            pcs = tmp['pc', hh, c0]
            for k in range(NC):
                w = vb[2 * jv + hh, r, pl.ds(8 * (c0 + k), 8), :]
                vf = pltpu.bitcast(w, jnp.bfloat16).astype(jnp.float32)
                u = vf[0:8] * pcs[2 * k] + vf[8:16] * pcs[2 * k + 1]
                acc = u if acc is None else acc + u
            if c0 > 0:
                acc = tmp['oacc', hh, r, c0] + acc
            buf[pl.ds(zo_w + DH * hh + 8 * r, 8), :] = acc

        fn = dict(bln=b_load_next, qmm=q_mm, qexpl=q_exp_load, qexps=q_exp_store, bl=b_load, qk=qk_unit,
                  sml=sm_load, sms=sm_store, worow=wo_row, wof=wo_fold, ol=out_load, wo=wo_mm,
                  pl=p_load, al=acc_load, pv=pv_unit)
        stage_of = dict(bln='qk', qmm='q', qexpl='q', qexps='q', bl='qk', qk='qk', sml='sm', sms='sm', worow='wo',
                        wof='wo', ol='wo', wo='wo', pl='pv', al='pv', pv='pv')

        late = grp is not None and grp[1] == 1 and bases is not None
        start = cfg.get('start2' if late else 'start', 0.12)
        span = cfg.get('span2' if late else 'span', 0.9)
        pos = []
        if pv:
            blocks = [(hh, c0) for hh in range(2) for c0 in range(0, 16, NC)]
            units = [('pv', hh, r, c0) for (hh, c0) in blocks for r in range(24)]
            n = len(units)
            for i, it in enumerate(units):
                pos.append(((i + 0.5) / n, it))
                if it[3] > 0:
                    pos.append(((i + 0.5 - cfg.get('aahead', 4)) / n - 1e-7, ('al',) + it[1:]))
            for b, (hh, c0) in enumerate(blocks):
                pos.append((b / len(blocks) - cfg.get('pahead', 0.02) if b else -0.9, ('pl', hh, c0)))
        qk_items = [(('qk', hh, cc, jj), 24) for hh in range(2) for cc in range(2) for jj in range(8)]
        if grp is None:
            q_items = [(('qmm', g), 16) for g in range(10)]
        else:
            q_items = [(('qmm', g), 24) for g in range(5 * grp[1], 5 * grp[1] + 5)]
        do_exp = grp is None or grp[1] == 1
        wo_items = [(('wo', v), 24) for v in range(5)]
        qa, wa = cfg.get('q_at', 0), cfg.get('wo_at', 12)
        mx = list(qk_items)
        e_items = [(('qexpl',), 16)] if do_exp else []
        ins = sorted(((qa, 0, q_items), (cfg.get('e_at', 8), 1, e_items), (wa, 2, wo_items)), reverse=True)
        for at, _, items in ins:
            mx[at:at] = items
        tot = float(sum(w for _, w in mx))
        acc = 0
        for it, w in mx:
            acc += w
            p_ = start + (span - start) * acc / tot
            pos.append((p_, it))
            if it[0] == 'wo':
                pos.append((p_ - cfg.get('oahead', 0.03), ('ol', it[1])))
        if q and do_exp:
            pos.append((cfg.get('qexp', 0.6), ('qexps',)))
        if qk:
            pos.append((-1.0, ('bl',)))
        if next_bases:
            pos.append((cfg.get('bln', 0.7), ('bln',)))
        if sm:
            pos.append((-0.8, ('sml', 0)))
            pos.append((-0.7, ('sml', 1)))
            pos.append((cfg.get('sms', 0.6), ('sms', 0)))
            pos.append((cfg.get('sms', 0.6) + 0.01, ('sms', 1)))
        if wo:
            rows = [16 * b + r for r in range(16) for b in range(3)]
            wl0, wl1 = cfg.get('wl0', 0.0), cfg.get('wl1', 0.2)
            for i, k in enumerate(rows):
                pos.append((wl0 + (wl1 - wl0) * i / 48, ('worow', k)))
            pos.append((wl1 + 1e-4, ('wof',)))
        on = dict(q=q, qk=qk, sm=sm, pv=pv, wo=wo)
        pos = [e for e in pos if on[stage_of[e[1][0]]]]
        pos.sort(key=lambda e: e[0])
        if guard is None:
            for _, it in pos:
                fn[it[0]](*it[1:])
        else:
            for stage in ('q', 'qk', 'sm', 'pv', 'wo'):
                items = [it for _, it in pos if stage_of[it[0]] == stage]

                def run(items=items):
                    for it in items:
                        fn[it[0]](*it[1:])
                guard(stage, run)
        return tmp.get('nb')


def _kernel(x_hbm, zs_hbm, k_hbm, v_hbm, wq_hbm, wo_hbm, w3_hbm, w4_hbm, o_ref,
            kb, vb, wqb, wob, wos, w3b, w4b, buf, eb, xb, x_ref, zs, sems, *, w_rows, n_rows):
    k32 = k_hbm.bitcast(jnp.uint32)
    v32 = v_hbm.bitcast(jnp.uint32)
    r0 = n_rows - w_rows

    def cp_k(j):
        return pltpu.make_async_copy(
            k32.at[pl.ds(2 * j, 2), :, pl.ds(r0, w_rows), :], kb.at[pl.ds(2 * j, 2)], sems.at[j])

    def cp_v(j):
        return pltpu.make_async_copy(
            v32.at[pl.ds(2 * j, 2), :, pl.ds(r0, w_rows), :], vb.at[pl.ds(2 * j, 2)], sems.at[NP + j])

    def cp_wo(j):
        return pltpu.make_async_copy(
            wo_hbm.at[pl.ds(2 * DH * j, 2 * DH), :], wos.at[j & 3], sems.at[2 * NP + j])

    cp_wq = pltpu.make_async_copy(wq_hbm.bitcast(jnp.uint32), wqb, sems.at[3 * NP])
    cp_w3 = pltpu.make_async_copy(w3_hbm, w3b, sems.at[3 * NP + 1])
    cw = F // W4_CHUNKS

    def cp_w4(c):
        return pltpu.make_async_copy(w4_hbm.at[pl.ds(cw * c, cw)], w4b.at[pl.ds(cw * c, cw)],
                                     sems.at[3 * NP + 4 + c])

    cp_x = pltpu.make_async_copy(x_hbm, x_ref, sems.at[3 * NP + 2])
    cp_z = pltpu.make_async_copy(zs_hbm, zs, sems.at[3 * NP + 3])

    def valid(j):
        return jnp.logical_and(j >= 0, j < NP)

    def clamp(j):
        return jnp.clip(j, 0, NP - 1)

    def start_group(t):
        for cp, j in ((cp_k, t), (cp_v, t - 2), (cp_wo, t - 3)):
            if isinstance(j, int):
                if 0 <= j < NP:
                    cp(j).start()
            else:
                @pl.when(valid(j))
                def _(cp=cp, j=j):
                    cp(clamp(j)).start()

    def wait_group(t):
        for cp, j in ((cp_k, t), (cp_v, t - 2), (cp_wo, t - 3)):
            @pl.when(valid(j))
            def _(cp=cp, j=j):
                cp(clamp(j)).wait()

    cp_wq.start()
    cp_x.start()
    cp_z.start()
    for t in (0, 1):
        start_group(t)
    cp_z.wait()
    cp_x.wait()

    att = _Attn(kb, vb, wqb, wob, buf, zs, eb, xb)
    att.init_expander()

    def attention_streaming(x):
        att.set_x(x)
        att.zero_out()
        cp_wq.wait()

        def body(t, carry):
            wait_group(t)

            @pl.when(t >= 3)
            def _():
                j = t - 3
                for v in range(D // LANES):
                    wob[j, v] = pltpu.bitcast(wos[j & 3, :, pl.ds(LANES * v, LANES)], jnp.uint32)
            start_group(t + 3)

            @pl.when(t == NP - 1)
            def _():
                cp_w3.start()
                for c in range(W4_CHUNKS):
                    cp_w4(c).start()

            first = dict(q=-1, qk=0, sm=1, pv=2, wo=3)

            def guard(stage, run):
                pl.when(jnp.logical_and(t >= first[stage], t < first[stage] + NP))(run)
            att.step(t, guard=guard)
            return carry
        jax.lax.fori_loop(-1, NP + 3, body, 0)
        return x + att.read_out()

    def attention_resident(x):
        att.set_x(x)
        att.zero_out()
        att.step(-2, qk=False, sm=False, pv=False, wo=False, grp=(-1, 0))
        att.step(-1, qk=False, sm=False, pv=False, wo=False, grp=(-1, 1))
        nb = att.step(0, sm=False, pv=False, wo=False, grp=(0, 0), next_bases=True)
        att.step(1, pv=False, wo=False, grp=(0, 1), bases=nb)

        def body(b, carry):
            nb = att.step(2 * b, clamp_idx=True, grp=(b, 0), next_bases=True)
            att.step(2 * b + 1, clamp_idx=True, grp=(b, 1), bases=nb)
            return carry
        jax.lax.fori_loop(1, NP // 2 + 1, body, 0)
        att.step(NP + 2, q=False, qk=False, sm=False, pv=False)
        return x + att.read_out()

    def mixer(x, first):
        y = _ln(x)
        z = jnp.broadcast_to(_ln_centred(y), (16, D)).astype(jnp.bfloat16)
        if first:
            cp_w3.wait()
        h = jnp.dot(z, w3b[...], preferred_element_type=jnp.float32)
        h = jax.nn.gelu(h, approximate=True).astype(jnp.bfloat16)
        h2 = None
        for c in range(W4_CHUNKS):
            if first:
                cp_w4(c).wait()
            d = jnp.dot(h[:, cw * c:cw * (c + 1)], w4b[pl.ds(cw * c, cw), :], preferred_element_type=jnp.float32)[0:8]
            h2 = d if h2 is None else h2 + d
        return x + (y + h2[0:1])

    x = x_ref[...].astype(jnp.float32)
    x = attention_streaming(x)
    x = mixer(x, True)
    x = attention_resident(x)
    x = mixer(x, False)
    o_ref[...] = x.astype(o_ref.dtype)


def _tile_view(c):
    _, h, s, dh = c.shape
    return (c.reshape(h, s // LANES, LANES, dh // 8, 8)
            .transpose(0, 3, 1, 4, 2)
            .reshape(h, dh // 8, s // LANES * 8, LANES))


@jax.jit
def pallas_interleave_layers__sliding_block_cached__mixer_s_mlp__decode_kernel(
    A_x: jax.Array,
    A_k_cache: jax.Array,
    A_v_cache: jax.Array,
    A_wq: jax.Array,
    A_wo: jax.Array,
    B_x: jax.Array,
    B_w1: jax.Array,
    B_w2: jax.Array,
    B_w3: jax.Array,
    B_w4: jax.Array,
):
    del B_x, B_w1, B_w2
    s = A_k_cache.shape[2]
    w = min(4096, max(256, s // 4))
    w_rows = w // LANES * 4
    n_rows = s // LANES * 4
    kk = _tile_view(A_k_cache)
    vv = _tile_view(A_v_cache)
    wq_t = (A_wq.reshape(D // 8, 8, H * DH // LANES, LANES).transpose(0, 2, 1, 3)
            .reshape(D // 8, H * DH // LANES * 8, LANES))
    any_spec = pl.BlockSpec(memory_space=pl.ANY)
    out = pl.pallas_call(
        functools.partial(_kernel, w_rows=w_rows, n_rows=n_rows),
        out_shape=jax.ShapeDtypeStruct((1, D), A_x.dtype),
        in_specs=[any_spec] * 8,
        out_specs=pl.BlockSpec(memory_space=pltpu.VMEM),
        scratch_shapes=[
            pltpu.VMEM((H, 24, w_rows, LANES), jnp.uint32),
            pltpu.VMEM((H, 24, w_rows, LANES), jnp.uint32),
            pltpu.VMEM((D // 8, H * DH // LANES * 4, LANES), jnp.uint32),
            pltpu.VMEM((NP, D // LANES, DH, LANES), jnp.uint32),
            pltpu.VMEM((4, 2 * DH, D), jnp.bfloat16),
            pltpu.VMEM((D, F), jnp.bfloat16),
            pltpu.VMEM((F, D), jnp.bfloat16),
            pltpu.VMEM((R_END, LANES), jnp.float32),
            pltpu.VMEM((2, LANES // 2, LANES), jnp.uint32),
            pltpu.VMEM((10, 8, LANES), jnp.uint32),
            pltpu.VMEM((1, D), A_x.dtype),
            pltpu.SMEM((8,), jnp.int32),
            pltpu.SemaphoreType.DMA((3 * NP + 4 + W4_CHUNKS,)),
        ],
        compiler_params=pltpu.CompilerParams(vmem_limit_bytes=127 * 1024 * 1024),
    )(A_x.reshape(1, D), jnp.zeros((8,), jnp.int32), kk, vv, wq_t, A_wo, B_w3, B_w4)
    return out.reshape(A_x.shape)
```

```python
import functools

import jax
import jax.numpy as jnp
import jax.experimental.pallas as pl
import jax.experimental.pallas.tpu as pltpu

H = 32
DH = 192
D = 640
F = 1536
LANES = 128
NP = H // 2
EPS = 1e-5


def _ln(x):
    m = jnp.mean(x, axis=-1, keepdims=True)
    d = x - m
    v = jnp.mean(d * d, axis=-1, keepdims=True)
    return d * jax.lax.rsqrt(v + EPS)


def _ln_centred(y):
    m = jnp.mean(y, axis=-1, keepdims=True)
    v = jnp.mean(y * y, axis=-1, keepdims=True) - m * m
    return (y - m) * jax.lax.rsqrt(v + EPS)


R_O, R_S, R_B, R_Q, R_OUT, R_P, R_END = 0, 768, 896, 992, 1016, 1096, 1224
W4_CHUNKS = 4
KVG = 2
CFG = dict(q_at=0, e_at=16, wo_at=24, start=0.13, span=0.89, start2=0.16, span2=0.86, bln=0.5,
           sms=0.6, wl0=0.0, wl1=0.15, aahead=2, pahead=0.02, nc=16, qexp=0.8, oahead=0.03, peel=True,
           tail=dict(nc=16, wo_at=32, start=0.3, span=0.6, sms=0.3),
           flags={"XLA_TPU_EVENLY_DISTRIBUTE_CRITICAL_NODES": True})


def _f2u(x):
    return pltpu.bitcast(x, jnp.uint32)


def _u2f(x):
    return pltpu.bitcast(x, jnp.float32)


class _Attn:
    def __init__(self, kb, vb, wqb, wob, buf, zs, eb, xb):
        self.kb, self.vb, self.wqb, self.wob, self.buf = kb, vb, wqb, wob, buf
        self.eb, self.xb = eb, xb
        self.z = [pl.multiple_of(zs[k], 8) for k in range(8)]
        self.lane = jax.lax.broadcasted_iota(jnp.int32, (8, LANES), 1)
        self.sub = jax.lax.broadcasted_iota(jnp.int32, (8, LANES), 0)
        self.half = jnp.where((self.lane & 8) != 0, jnp.uint32(0xFFFF0000), jnp.uint32(0x0000FFFF))

    def init_expander(self):
        src = jax.lax.broadcasted_iota(jnp.int32, (LANES, LANES), 0)
        dst = jax.lax.broadcasted_iota(jnp.int32, (LANES, LANES), 1)
        for h in range(2):
            e = jnp.where(src == 64 * h + 8 * (dst >> 4) + (dst & 7), 1.0, 0.0).astype(jnp.bfloat16)
            self.eb[h] = pltpu.bitcast(e, jnp.uint32)

    def expand(self, rows):
        lhs = jnp.concatenate([rows, rows], axis=0).astype(jnp.bfloat16)
        outs = []
        for h in range(2):
            e = pltpu.bitcast(self.eb[h], jnp.bfloat16)
            ex = jnp.dot(lhs, e, preferred_element_type=jnp.float32)[0:8]
            b = _f2u(ex)
            outs.append((b | (b >> 16)) & self.half)
        return outs

    def set_x(self, x):
        xn = _ln(x).astype(jnp.bfloat16).astype(jnp.float32)
        rows = jnp.zeros((8, LANES), jnp.float32)
        for v in range(D // LANES):
            rows = jnp.where(self.sub == v, jnp.broadcast_to(xn[:, LANES * v:LANES * (v + 1)], (8, LANES)), rows)
        ex = self.expand(rows)
        for g in range(10):
            self.xb[g] = jnp.broadcast_to(ex[g % 2][g // 2:g // 2 + 1, :], (8, LANES))

    def zero_out(self):
        self.buf[pl.ds(self.z[0] + R_OUT, 80), :] = jnp.zeros((80, LANES), jnp.float32)

    def read_out(self):
        o = jnp.concatenate(
            [self.buf[pl.ds(self.z[0] + R_OUT + 16 * v, 16), :] for v in range(5)], axis=1)
        return jnp.sum(o, axis=0, keepdims=True)

    def step(self, t, *, q=True, qk=True, sm=True, pv=True, wo=True, guard=None, cfg=None,
             clamp_idx=False, grp=None, bases=None, next_bases=False):
        cfg = cfg or CFG
        buf, z, lane, sub, half = self.buf, self.z, self.lane, self.sub, self.half
        kb, vb, wqb, wob = self.kb, self.vb, self.wqb, self.wob
        par = t & 1 if grp is None else grp[1]
        npar = 1 - par
        zq = z[0] + R_Q
        bpar = par if grp is None else grp[0] & 1
        zb_w = z[1] + R_B + bpar * 16
        zb_r = z[1] + R_B + (1 - bpar) * 16
        zs_w = z[2] + R_S + par * 64
        zs_r = z[3] + R_S + npar * 64
        zp_w = z[4] + R_P + par * 64
        zp_r = z[5] + R_P + npar * 64
        zo_w = z[6] + R_O + par * 384
        zo_r = z[7] + R_O + npar * 384
        zout = z[0] + R_OUT
        scale = DH ** -0.5
        tmp = {}
        NC = cfg.get('nc', 8)
        if clamp_idx:
            jq, jk = jnp.minimum(t + 1, NP - 1), jnp.minimum(t, NP - 1)
            jv, jo = t - 2, jnp.maximum(t - 3, 0)
        else:
            jq, jk, jv, jo = t + 1, t, t - 2, t - 3

        def q_mm(g):
            xbase = self.xb[g]
            d = None
            if grp is None:
                c0, na = 3 * jq >> 1, 2
            else:
                gq = grp[0] + 1
                c0, na = 3 * (jnp.minimum(gq, NP // 2 - 1) if clamp_idx else gq), 3
            for a in range(na):
                lhs = pltpu.bitcast(jnp.where(sub == a, xbase, jnp.uint32(0)), jnp.bfloat16)
                w = wqb[pl.ds(8 * g, 8), pl.ds(pl.multiple_of(8 * (c0 + a), 8), 8), :]
                w = pltpu.bitcast(w, jnp.bfloat16).reshape(128, LANES)
                dd = jnp.dot(lhs, w, preferred_element_type=jnp.float32)[0:8]
                d = dd if d is None else d + dd
            if g > 0:
                d = (tmp['q'] if 'q' in tmp else buf[pl.ds(zq, 8), :]) + d
            tmp['q'] = d
            buf[pl.ds(zq, 8), :] = d

        def q_exp_load():
            tmp['b'] = self.expand(buf[pl.ds(zq, 8), :].astype(jnp.bfloat16).astype(jnp.float32))

        def q_exp_store():
            for h in range(2):
                buf[pl.ds(zb_w + 8 * h, 8), :] = _u2f(tmp['b'][h])

        def load_bases(odd):
            return [jnp.broadcast_to(_f2u(buf[pl.ds(zb_r + 8 * (s % 2) + odd + s // 2, 1), :]), (8, LANES))
                    for s in range(6)]

        def b_load():
            if bases is not None:
                tmp['bases'] = bases
            else:
                tmp['bases'] = load_bases(jk & 1 if grp is None else 3 * grp[1])

        def b_load_next():
            tmp['nb'] = load_bases(3)

        def qk_unit(hh, cc, jj):
            d = None
            for g in range(3):
                lhs = pltpu.bitcast(jnp.where(sub == jj, tmp['bases'][3 * hh + g], jnp.uint32(0)), jnp.bfloat16)
                w = kb[2 * jk + hh, pl.ds(8 * g, 8), pl.ds(8 * (cc * 8 + jj), 8), :]
                w = pltpu.bitcast(w, jnp.bfloat16).reshape(128, LANES)
                dd = jnp.dot(lhs, w, preferred_element_type=jnp.float32)
                d = dd if d is None else d + dd
            if jj > 0:
                d = tmp['sacc'] + d
            tmp['sacc'] = d
            buf[pl.ds(zs_w + 32 * hh + 16 * cc, 16), :] = d

        def sm_load(hh):
            s = buf[pl.ds(zs_r + 32 * hh, 32), :] * scale
            m = jnp.max(jnp.max(s, axis=1, keepdims=True), axis=0, keepdims=True)
            e = jnp.exp(s - m)
            l = jnp.sum(jnp.sum(e, axis=1, keepdims=True), axis=0, keepdims=True)
            tmp['p', hh] = e * (1.0 / l)

        def sm_store(hh):
            buf[pl.ds(zp_w + 32 * hh, 32), :] = tmp['p', hh]

        def wo_row(k):
            tmp['orow', k] = buf[pl.ds(zo_r + 8 * k, 8), :]

        def wo_fold():
            ot = jnp.concatenate([tmp['orow', k] for k in range(48)], axis=0).T
            tmp['fold'] = ot.reshape(8, 16, 2 * DH).sum(axis=0).astype(jnp.bfloat16)

        def out_load(v):
            tmp['out', v] = buf[pl.ds(zout + 16 * v, 16), :]

        def wo_mm(v):
            w = pltpu.bitcast(wob[jo, v], jnp.bfloat16)
            r = jnp.dot(tmp['fold'], w, preferred_element_type=jnp.float32)
            if clamp_idx:
                r = jnp.where(t >= 3, r, 0.0)
            buf[pl.ds(zout + 16 * v, 16), :] = tmp['out', v] + r

        def p_load(hh, c0):
            tmp['pc', hh, c0] = [jnp.broadcast_to(buf[pl.ds(zp_r + 32 * hh + c, 1), :], (8, LANES))
                                 for c in range(2 * c0, 2 * (c0 + NC))]

        def acc_load(hh, r, c0):
            tmp['oacc', hh, r, c0] = buf[pl.ds(zo_w + DH * hh + 8 * r, 8), :]

        def pv_unit(hh, r, c0):
            acc = None
            pcs = tmp['pc', hh, c0]
            for k in range(NC):
                w = vb[2 * jv + hh, r, pl.ds(8 * (c0 + k), 8), :]
                vf = pltpu.bitcast(w, jnp.bfloat16).astype(jnp.float32)
                u = vf[0:8] * pcs[2 * k] + vf[8:16] * pcs[2 * k + 1]
                acc = u if acc is None else acc + u
            if c0 > 0:
                acc = tmp['oacc', hh, r, c0] + acc
            buf[pl.ds(zo_w + DH * hh + 8 * r, 8), :] = acc

        fn = dict(bln=b_load_next, qmm=q_mm, qexpl=q_exp_load, qexps=q_exp_store, bl=b_load, qk=qk_unit,
                  sml=sm_load, sms=sm_store, worow=wo_row, wof=wo_fold, ol=out_load, wo=wo_mm,
                  pl=p_load, al=acc_load, pv=pv_unit)
        stage_of = dict(bln='qk', qmm='q', qexpl='q', qexps='q', bl='qk', qk='qk', sml='sm', sms='sm', worow='wo',
                        wof='wo', ol='wo', wo='wo', pl='pv', al='pv', pv='pv')

        late = grp is not None and grp[1] == 1 and bases is not None
        start = cfg.get('start2' if late else 'start', 0.12)
        span = cfg.get('span2' if late else 'span', 0.9)
        pos = []
        if pv:
            blocks = [(hh, c0) for hh in range(2) for c0 in range(0, 16, NC)]
            units = [('pv', hh, r, c0) for (hh, c0) in blocks for r in range(24)]
            n = len(units)
            for i, it in enumerate(units):
                pos.append(((i + 0.5) / n, it))
                if it[3] > 0:
                    pos.append(((i + 0.5 - cfg.get('aahead', 4)) / n - 1e-7, ('al',) + it[1:]))
            for b, (hh, c0) in enumerate(blocks):
                pos.append((b / len(blocks) - cfg.get('pahead', 0.02) if b else -0.9, ('pl', hh, c0)))
        qk_items = [(('qk', hh, cc, jj), 24) for hh in range(2) for cc in range(2) for jj in range(8)]
        if grp is None:
            q_items = [(('qmm', g), 16) for g in range(10)]
        else:
            q_items = [(('qmm', g), 24) for g in range(5 * grp[1], 5 * grp[1] + 5)]
        do_exp = grp is None or grp[1] == 1
        wo_items = [(('wo', v), 24) for v in range(5)]
        qa, wa = cfg.get('q_at', 0), cfg.get('wo_at', 12)
        mx = list(qk_items)
        e_items = [(('qexpl',), 16)] if do_exp else []
        ins = sorted(((qa, 0, q_items), (cfg.get('e_at', 8), 1, e_items), (wa, 2, wo_items)), reverse=True)
        for at, _, items in ins:
            mx[at:at] = items
        tot = float(sum(w for _, w in mx))
        acc = 0
        for it, w in mx:
            acc += w
            p_ = start + (span - start) * acc / tot
            pos.append((p_, it))
            if it[0] == 'wo':
                pos.append((p_ - cfg.get('oahead', 0.03), ('ol', it[1])))
        if q and do_exp:
            pos.append((cfg.get('qexp', 0.6), ('qexps',)))
        if qk:
            pos.append((-1.0, ('bl',)))
        if next_bases:
            pos.append((cfg.get('bln', 0.7), ('bln',)))
        if sm:
            pos.append((-0.8, ('sml', 0)))
            pos.append((-0.7, ('sml', 1)))
            pos.append((cfg.get('sms', 0.6), ('sms', 0)))
            pos.append((cfg.get('sms', 0.6) + 0.01, ('sms', 1)))
        if wo:
            rows = [16 * b + r for r in range(16) for b in range(3)]
            wl0, wl1 = cfg.get('wl0', 0.0), cfg.get('wl1', 0.2)
            for i, k in enumerate(rows):
                pos.append((wl0 + (wl1 - wl0) * i / 48, ('worow', k)))
            pos.append((wl1 + 1e-4, ('wof',)))
        on = dict(q=q, qk=qk, sm=sm, pv=pv, wo=wo)
        pos = [e for e in pos if on[stage_of[e[1][0]]]]
        pos.sort(key=lambda e: e[0])
        if guard is None:
            for _, it in pos:
                fn[it[0]](*it[1:])
        else:
            for stage in ('q', 'qk', 'sm', 'pv', 'wo'):
                items = [it for _, it in pos if stage_of[it[0]] == stage]

                def run(items=items):
                    for it in items:
                        fn[it[0]](*it[1:])
                guard(stage, run)
        return tmp.get('nb')


def _kernel(x_hbm, zs_hbm, k_hbm, v_hbm, wq_hbm, wo_hbm, w3_hbm, w4_hbm, o_ref,
            kb, vb, wqb, wob, wos, w3b, w4b, buf, eb, xb, x_ref, zs, sems, *, w_rows, n_rows):
    k32 = k_hbm.bitcast(jnp.uint32)
    v32 = v_hbm.bitcast(jnp.uint32)
    r0 = n_rows - w_rows

    def cp_k(j):
        return pltpu.make_async_copy(
            k32.at[pl.ds(2 * j, 2 * KVG), :, pl.ds(r0, w_rows), :], kb.at[pl.ds(2 * j, 2 * KVG)], sems.at[j])

    def cp_v(j):
        return pltpu.make_async_copy(
            v32.at[pl.ds(2 * j, 2 * KVG), :, pl.ds(r0, w_rows), :], vb.at[pl.ds(2 * j, 2 * KVG)], sems.at[NP + j])

    def cp_wo(j):
        return pltpu.make_async_copy(
            wo_hbm.at[pl.ds(2 * DH * j, 2 * DH), :], wos.at[j & 3], sems.at[2 * NP + j])

    cp_wq = pltpu.make_async_copy(wq_hbm.bitcast(jnp.uint32), wqb, sems.at[3 * NP])
    cp_w3 = pltpu.make_async_copy(w3_hbm, w3b, sems.at[3 * NP + 1])
    cw = F // W4_CHUNKS

    def cp_w4(c):
        return pltpu.make_async_copy(w4_hbm.at[pl.ds(cw * c, cw)], w4b.at[pl.ds(cw * c, cw)],
                                     sems.at[3 * NP + 4 + c])

    cp_x = pltpu.make_async_copy(x_hbm, x_ref, sems.at[3 * NP + 2])
    cp_z = pltpu.make_async_copy(zs_hbm, zs, sems.at[3 * NP + 3])

    def valid(j):
        return jnp.logical_and(j >= 0, j < NP)

    def clamp(j):
        return jnp.clip(j, 0, NP - 1)

    def start_group(t):
        for cp, j, g in ((cp_k, t, KVG), (cp_v, t - 2, KVG), (cp_wo, t - 3, 1)):
            if isinstance(j, int):
                if 0 <= j < NP and j % g == 0:
                    cp(j).start()
            else:
                @pl.when(jnp.logical_and(valid(j), (j & (g - 1)) == 0))
                def _(cp=cp, j=j):
                    cp(clamp(j) & -g).start()

    def wait_group(t):
        for cp, j, g in ((cp_k, t, KVG), (cp_v, t - 2, KVG), (cp_wo, t - 3, 1)):
            @pl.when(jnp.logical_and(valid(j), (j & (g - 1)) == 0))
            def _(cp=cp, j=j):
                cp(clamp(j) & -g).wait()

    cp_wq.start()
    cp_x.start()
    cp_z.start()
    for t in (0, 1):
        start_group(t)
    cp_z.wait()
    cp_x.wait()

    att = _Attn(kb, vb, wqb, wob, buf, zs, eb, xb)
    att.init_expander()

    def attention_streaming(x):
        att.set_x(x)
        att.zero_out()
        cp_wq.wait()

        def body(t, carry):
            wait_group(t)

            @pl.when(t >= 3)
            def _():
                j = t - 3
                for v in range(D // LANES):
                    wob[j, v] = pltpu.bitcast(wos[j & 3, :, pl.ds(LANES * v, LANES)], jnp.uint32)
            start_group(t + 3)

            @pl.when(t == NP - 1)
            def _():
                cp_w3.start()
                for c in range(W4_CHUNKS):
                    cp_w4(c).start()

            first = dict(q=-1, qk=0, sm=1, pv=2, wo=3)

            def guard(stage, run):
                pl.when(jnp.logical_and(t >= first[stage], t < first[stage] + NP))(run)
            att.step(t, guard=guard)
            return carry
        jax.lax.fori_loop(-1, NP + 3, body, 0)
        return x + att.read_out()

    def attention_resident(x):
        att.set_x(x)
        att.zero_out()
        att.step(-2, qk=False, sm=False, pv=False, wo=False, grp=(-1, 0))
        att.step(-1, qk=False, sm=False, pv=False, wo=False, grp=(-1, 1))
        nb = att.step(0, sm=False, pv=False, wo=False, grp=(0, 0), next_bases=True)
        att.step(1, pv=False, wo=False, grp=(0, 1), bases=nb)

        def body(b, carry):
            nb = att.step(2 * b, clamp_idx=True, grp=(b, 0), next_bases=True)
            att.step(2 * b + 1, clamp_idx=True, grp=(b, 1), bases=nb)
            return carry
        if CFG.get('peel'):
            jax.lax.fori_loop(1, NP // 2, body, 0)

            @pl.when(zs[0] == 0)
            def _():
                att.step(NP, q=False, qk=False, cfg=CFG.get('tail'))
                att.step(NP + 1, q=False, qk=False, sm=False, cfg=CFG.get('tail'))
        else:
            jax.lax.fori_loop(1, NP // 2 + 1, body, 0)
        att.step(NP + 2, q=False, qk=False, sm=False, pv=False)
        return x + att.read_out()

    def mixer(x, first):
        y = _ln(x)
        z = jnp.broadcast_to(_ln_centred(y), (16, D)).astype(jnp.bfloat16)
        if first:
            cp_w3.wait()
        h = jnp.dot(z, w3b[...], preferred_element_type=jnp.float32)
        h = jax.nn.gelu(h, approximate=True).astype(jnp.bfloat16)
        h2 = None
        for c in range(W4_CHUNKS):
            if first:
                cp_w4(c).wait()
            d = jnp.dot(h[:, cw * c:cw * (c + 1)], w4b[pl.ds(cw * c, cw), :], preferred_element_type=jnp.float32)[0:8]
            h2 = d if h2 is None else h2 + d
        return x + (y + h2[0:1])

    x = x_ref[...].astype(jnp.float32)
    x = attention_streaming(x)
    x = mixer(x, True)
    x = attention_resident(x)
    x = mixer(x, False)
    o_ref[...] = x.astype(o_ref.dtype)


def _tile_view(c):
    _, h, s, dh = c.shape
    return (c.reshape(h, s // LANES, LANES, dh // 8, 8)
            .transpose(0, 3, 1, 4, 2)
            .reshape(h, dh // 8, s // LANES * 8, LANES))


@jax.jit
def pallas_interleave_layers__sliding_block_cached__mixer_s_mlp__decode_kernel(
    A_x: jax.Array,
    A_k_cache: jax.Array,
    A_v_cache: jax.Array,
    A_wq: jax.Array,
    A_wo: jax.Array,
    B_x: jax.Array,
    B_w1: jax.Array,
    B_w2: jax.Array,
    B_w3: jax.Array,
    B_w4: jax.Array,
):
    del B_x, B_w1, B_w2
    s = A_k_cache.shape[2]
    w = min(4096, max(256, s // 4))
    w_rows = w // LANES * 4
    n_rows = s // LANES * 4
    kk = _tile_view(A_k_cache)
    vv = _tile_view(A_v_cache)
    wq_t = (A_wq.reshape(D // 8, 8, H * DH // LANES, LANES).transpose(0, 2, 1, 3)
            .reshape(D // 8, H * DH // LANES * 8, LANES))
    any_spec = pl.BlockSpec(memory_space=pl.ANY)
    out = pl.pallas_call(
        functools.partial(_kernel, w_rows=w_rows, n_rows=n_rows),
        out_shape=jax.ShapeDtypeStruct((1, D), A_x.dtype),
        in_specs=[any_spec] * 8,
        out_specs=pl.BlockSpec(memory_space=pltpu.VMEM),
        scratch_shapes=[
            pltpu.VMEM((H, 24, w_rows, LANES), jnp.uint32),
            pltpu.VMEM((H, 24, w_rows, LANES), jnp.uint32),
            pltpu.VMEM((D // 8, H * DH // LANES * 4, LANES), jnp.uint32),
            pltpu.VMEM((NP, D // LANES, DH, LANES), jnp.uint32),
            pltpu.VMEM((4, 2 * DH, D), jnp.bfloat16),
            pltpu.VMEM((D, F), jnp.bfloat16),
            pltpu.VMEM((F, D), jnp.bfloat16),
            pltpu.VMEM((R_END, LANES), jnp.float32),
            pltpu.VMEM((2, LANES // 2, LANES), jnp.uint32),
            pltpu.VMEM((10, 8, LANES), jnp.uint32),
            pltpu.VMEM((1, D), A_x.dtype),
            pltpu.SMEM((8,), jnp.int32),
            pltpu.SemaphoreType.DMA((3 * NP + 4 + W4_CHUNKS,)),
        ],
        compiler_params=pltpu.CompilerParams(vmem_limit_bytes=127 * 1024 * 1024,
                                             flags=CFG.get('flags')),
    )(A_x.reshape(1, D), jnp.zeros((8,), jnp.int32), kk, vv, wq_t, A_wo, B_w3, B_w4)
    return out.reshape(A_x.shape)
```

```python
import functools

import jax
import jax.numpy as jnp
import jax.experimental.pallas as pl
import jax.experimental.pallas.tpu as pltpu


H = 32
DH = 192
D = 640
F = 1536
LANES = 128
NP = H // 2
EPS = 1e-5


def _ln(x):
    m = jnp.mean(x, axis=-1, keepdims=True)
    d = x - m
    v = jnp.mean(d * d, axis=-1, keepdims=True)
    return d * jax.lax.rsqrt(v + EPS)


def _ln_centred(y):
    m = jnp.mean(y, axis=-1, keepdims=True)
    v = jnp.mean(y * y, axis=-1, keepdims=True) - m * m
    return (y - m) * jax.lax.rsqrt(v + EPS)


R_O, R_S, R_B, R_Q, R_OUT, R_P, R_F, R_END = 0, 768, 896, 992, 1016, 1096, 1224, 1256
W4_CHUNKS = 4
KVG = 2
CFG = dict(q_at=0, e_at=16, wo_at=24, start=0.13, span=0.93, start2=0.14, span2=0.87, bln=0.9,
           sms=0.7, wl0=0.0, wl1=0.2, aahead=4, pahead=0.02, nc=16, qexp=0.9, oahead=0.08, peel=True, voff=True, ways=2,
           tail=dict(nc=16, wo_at=32, ways=4, start=0.5, span=0.9, sms=0.3, wl1=0.2, v0=0.0, v1=0.7, vof=0.97),
           flags={"XLA_TPU_EVENLY_DISTRIBUTE_CRITICAL_NODES": True})


def _f2u(x):
    return pltpu.bitcast(x, jnp.uint32)


def _u2f(x):
    return pltpu.bitcast(x, jnp.float32)


class _Attn:
    def __init__(self, kb, vb, wqb, wob, buf, zs, eb, xb):
        self.kb, self.vb, self.wqb, self.wob, self.buf = kb, vb, wqb, wob, buf
        self.eb, self.xb = eb, xb
        self.z = [pl.multiple_of(zs[k], 8) for k in range(8)]
        self.lane = jax.lax.broadcasted_iota(jnp.int32, (8, LANES), 1)
        self.sub = jax.lax.broadcasted_iota(jnp.int32, (8, LANES), 0)
        self.half = jnp.where((self.lane & 8) != 0, jnp.uint32(0xFFFF0000), jnp.uint32(0x0000FFFF))

    def init_expander(self):
        src = jax.lax.broadcasted_iota(jnp.int32, (LANES, LANES), 0)
        dst = jax.lax.broadcasted_iota(jnp.int32, (LANES, LANES), 1)
        for h in range(2):
            e = jnp.where(src == 64 * h + 8 * (dst >> 4) + (dst & 7), 1.0, 0.0).astype(jnp.bfloat16)
            self.eb[h] = pltpu.bitcast(e, jnp.uint32)
            et = jnp.where(dst == 64 * h + 8 * (src >> 4) + (src & 7), 1.0, 0.0).astype(jnp.bfloat16)
            self.eb[2 + h] = pltpu.bitcast(et, jnp.uint32)

    def expand(self, rows):
        lhs = jnp.concatenate([rows, rows], axis=0).astype(jnp.bfloat16)
        outs = []
        for h in range(2):
            e = pltpu.bitcast(self.eb[h], jnp.bfloat16)
            ex = jnp.dot(lhs, e, preferred_element_type=jnp.float32)[0:8]
            b = _f2u(ex)
            outs.append((b | (b >> 16)) & self.half)
        return outs

    def set_x(self, x):
        xn = _ln(x).astype(jnp.bfloat16).astype(jnp.float32)
        rows = jnp.zeros((8, LANES), jnp.float32)
        for v in range(D // LANES):
            rows = jnp.where(self.sub == v, jnp.broadcast_to(xn[:, LANES * v:LANES * (v + 1)], (8, LANES)), rows)
        ex = self.expand(rows)
        for g in range(10):
            self.xb[g] = jnp.broadcast_to(ex[g % 2][g // 2:g // 2 + 1, :], (8, LANES))

    def zero_out(self):
        self.buf[pl.ds(self.z[0] + R_OUT, 80), :] = jnp.zeros((80, LANES), jnp.float32)

    def read_out(self):
        o = jnp.concatenate(
            [self.buf[pl.ds(self.z[0] + R_OUT + 16 * v, 16), :] for v in range(5)], axis=1)
        return jnp.sum(o, axis=0, keepdims=True)

    def step(self, t, *, q=True, qk=True, sm=True, pv=True, wo=True, guard=None, cfg=None,
             clamp_idx=False, grp=None, bases=None, next_bases=False, voff=False, wo_off=False):
        cfg = cfg or CFG
        buf, z, sub = self.buf, self.z, self.sub
        kb, vb, wqb, wob = self.kb, self.vb, self.wqb, self.wob
        par = t & 1 if grp is None else grp[1]
        npar = 1 - par
        zq = z[0] + R_Q
        bpar = par if grp is None else grp[0] & 1
        zb_w = z[1] + R_B + bpar * 16
        zb_r = z[1] + R_B + (1 - bpar) * 16
        zs_w = z[2] + R_S + par * 64
        zs_r = z[3] + R_S + npar * 64
        zp_w = z[4] + R_P + par * 64
        zp_r = z[5] + R_P + npar * 64
        zo_w = z[6] + R_O + par * 384
        zo_r = z[7] + R_O + npar * 384
        zout = z[0] + R_OUT
        scale = DH ** -0.5
        tmp = {}
        NC = cfg.get('nc', 8)
        if clamp_idx:
            jq, jk = jnp.minimum(t + 1, NP - 1), jnp.minimum(t, NP - 1)
            jv, jo = t - 2, jnp.maximum(t - 3, 0)
        else:
            jq, jk, jv, jo = t + 1, t, t - 2, t - 3

        def q_mm(g):
            xbase = self.xb[g]
            d = None
            if grp is None:
                c0, na = 3 * jq >> 1, 2
            else:
                gq = grp[0] + 1
                c0, na = 3 * (jnp.minimum(gq, NP // 2 - 1) if clamp_idx else gq), 3
            for a in range(na):
                lhs = pltpu.bitcast(jnp.where(sub == a, xbase, jnp.uint32(0)), jnp.bfloat16)
                w = wqb[pl.ds(8 * g, 8), pl.ds(pl.multiple_of(8 * (c0 + a), 8), 8), :]
                w = pltpu.bitcast(w, jnp.bfloat16).reshape(128, LANES)
                dd = jnp.dot(lhs, w, preferred_element_type=jnp.float32)[0:8]
                d = dd if d is None else d + dd
            if g > 0:
                d = (tmp['q'] if 'q' in tmp else buf[pl.ds(zq, 8), :]) + d
            tmp['q'] = d
            buf[pl.ds(zq, 8), :] = d

        def q_exp_load():
            tmp['b'] = self.expand(buf[pl.ds(zq, 8), :].astype(jnp.bfloat16).astype(jnp.float32))

        def q_exp_store():
            for h in range(2):
                buf[pl.ds(zb_w + 8 * h, 8), :] = _u2f(tmp['b'][h])

        def load_bases(odd):
            return [jnp.broadcast_to(_f2u(buf[pl.ds(zb_r + 8 * (s % 2) + odd + s // 2, 1), :]), (8, LANES))
                    for s in range(6)]

        def b_load():
            if bases is not None:
                tmp['bases'] = bases
            else:
                tmp['bases'] = load_bases(jk & 1 if grp is None else 3 * grp[1])

        def b_load_next():
            tmp['nb'] = load_bases(3)

        def qk_unit(hh, cc, jj):
            d = None
            for g in range(3):
                lhs = pltpu.bitcast(jnp.where(sub == jj, tmp['bases'][3 * hh + g], jnp.uint32(0)), jnp.bfloat16)
                w = kb[2 * jk + hh, pl.ds(8 * g, 8), pl.ds(8 * (cc * 8 + jj), 8), :]
                w = pltpu.bitcast(w, jnp.bfloat16).reshape(128, LANES)
                dd = jnp.dot(lhs, w, preferred_element_type=jnp.float32)
                d = dd if d is None else d + dd
            if jj > 0:
                d = tmp['sacc'] + d
            tmp['sacc'] = d
            buf[pl.ds(zs_w + 32 * hh + 16 * cc, 16), :] = d

        def sm_load(hh):
            s = buf[pl.ds(zs_r + 32 * hh, 32), :] * scale
            m = jnp.max(jnp.max(s, axis=1, keepdims=True), axis=0, keepdims=True)
            e = jnp.exp(s - m)
            l = jnp.sum(jnp.sum(e, axis=1, keepdims=True), axis=0, keepdims=True)
            tmp['p', hh] = e * (1.0 / l)

        def sm_store(hh):
            buf[pl.ds(zp_w + 32 * hh, 32), :] = tmp['p', hh]

        def wo_row(k):
            tmp['orow', k] = buf[pl.ds(zo_r + 8 * k, 8), :]

        def wo_fold():
            if wo_off:
                ot = jnp.concatenate([tmp['orow', k] for k in range(32)], axis=0).T
                f = jnp.concatenate([ot.reshape(8, 16, 2 * LANES).sum(axis=0),
                                     buf[pl.ds(z[5] + R_F + npar * 16, 16), :]], axis=1)
            else:
                ot = jnp.concatenate([tmp['orow', k] for k in range(48)], axis=0).T
                f = ot.reshape(8, 16, 2 * DH).sum(axis=0)
            tmp['fold'] = f.astype(jnp.bfloat16)

        def vo_load():
            tmp['pw'] = [pltpu.bitcast(buf[pl.ds(zp_r + 32 + 16 * cc, 16), :].astype(jnp.bfloat16), jnp.uint32)
                         for cc in range(2)]

        def vo_unit(g, cc, jj):
            lhs = pltpu.bitcast(jnp.where(sub == jj, tmp['pw'][cc], jnp.uint32(0)), jnp.bfloat16)
            w = vb[2 * jv + 1, pl.ds(8 * g, 8), pl.ds(8 * (cc * 8 + jj), 8), :]
            w = pltpu.bitcast(w, jnp.bfloat16).reshape(128, LANES)
            d = jax.lax.dot_general(lhs, w, (((1,), (1,)), ((), ())), preferred_element_type=jnp.float32)
            tmp['vo', g] = d if (cc == 0 and jj == 0) else tmp['vo', g] + d

        def vo_fin():
            row = jax.lax.broadcasted_iota(jnp.int32, (16, LANES), 0)
            col = jax.lax.broadcasted_iota(jnp.int32, (16, LANES), 1)
            keep = (row & 1) == ((col >> 3) & 1)
            f = None
            for g in (1, 2):
                lhs = jnp.where(keep, tmp['vo', g], 0.0).astype(jnp.bfloat16)
                d = jnp.dot(lhs, pltpu.bitcast(self.eb[1 + g], jnp.bfloat16), preferred_element_type=jnp.float32)
                f = d if f is None else f + d
            buf[pl.ds(z[4] + R_F + par * 16, 16), :] = f

        def out_load(v):
            tmp['out', v] = buf[pl.ds(zout + 16 * v, 16), :]

        def wo_mm(v):
            w = pltpu.bitcast(wob[jo, v], jnp.bfloat16)
            r = jnp.dot(tmp['fold'], w, preferred_element_type=jnp.float32)
            if clamp_idx:
                r = jnp.where(t >= 3, r, 0.0)
            buf[pl.ds(zout + 16 * v, 16), :] = tmp['out', v] + r

        def p_load(hh, c0):
            tmp['pc', hh, c0] = [jnp.broadcast_to(buf[pl.ds(zp_r + 32 * hh + c, 1), :], (8, LANES))
                                 for c in range(2 * c0, 2 * (c0 + NC))]

        def acc_load(hh, r, c0):
            tmp['oacc', hh, r, c0] = buf[pl.ds(zo_w + DH * hh + 8 * r, 8), :]

        def pv_unit(hh, r, c0):
            us = []
            pcs = tmp['pc', hh, c0]
            for k in range(NC):
                w = vb[2 * jv + hh, r, pl.ds(8 * (c0 + k), 8), :]
                vf = pltpu.bitcast(w, jnp.bfloat16).astype(jnp.float32)
                us.append(vf[0:8] * pcs[2 * k] + vf[8:16] * pcs[2 * k + 1])
            ways = cfg.get('ways', 1)
            parts = []
            for w_ in range(ways):
                acc = None
                for u in us[w_::ways]:
                    acc = u if acc is None else acc + u
                parts.append(acc)
            while len(parts) > 1:
                parts = [parts[i] + parts[i + 1] for i in range(0, len(parts), 2)]
            acc = parts[0]
            if c0 > 0:
                acc = tmp['oacc', hh, r, c0] + acc
            buf[pl.ds(zo_w + DH * hh + 8 * r, 8), :] = acc

        fn = dict(vol=vo_load, vo=vo_unit, vof=vo_fin, bln=b_load_next, qmm=q_mm, qexpl=q_exp_load, qexps=q_exp_store, bl=b_load, qk=qk_unit,
                  sml=sm_load, sms=sm_store, worow=wo_row, wof=wo_fold, ol=out_load, wo=wo_mm,
                  pl=p_load, al=acc_load, pv=pv_unit)
        stage_of = dict(vol='pv', vo='pv', vof='pv', bln='qk', qmm='q', qexpl='q', qexps='q', bl='qk', qk='qk', sml='sm', sms='sm', worow='wo',
                        wof='wo', ol='wo', wo='wo', pl='pv', al='pv', pv='pv')

        late = grp is not None and grp[1] == 1 and bases is not None
        start = cfg.get('start2' if late else 'start', 0.12)
        span = cfg.get('span2' if late else 'span', 0.9)
        pos = []
        if pv:
            blocks = [(hh, c0) for hh in range(2) for c0 in range(0, 16, NC)]
            units = [('pv', hh, r, c0) for (hh, c0) in blocks for r in range(24)
                     if not (voff and hh == 1 and r >= 8)]
            n = len(units)
            if voff:
                vos = [('vo', g, cc, jj) for g in (1, 2) for cc in range(2) for jj in range(8)]
                v0, v1 = cfg.get('v0', 0.05), cfg.get('v1', 0.75)
                pos.append((-0.95, ('vol',)))
                for i, it in enumerate(vos):
                    pos.append((v0 + (v1 - v0) * i / len(vos), it))
                pos.append((cfg.get('vof', 0.95), ('vof',)))
            for i, it in enumerate(units):
                pos.append(((i + 0.5) / n, it))
                if it[3] > 0:
                    pos.append(((i + 0.5 - cfg.get('aahead', 4)) / n - 1e-7, ('al',) + it[1:]))
            for b, (hh, c0) in enumerate(blocks):
                first = [i for i, it in enumerate(units) if (it[1], it[3]) == (hh, c0)][0]
                pos.append((first / n - cfg.get('pahead', 0.02) if b else -0.9, ('pl', hh, c0)))
        qk_items = [(('qk', hh, cc, jj), 24) for hh in range(2) for cc in range(2) for jj in range(8)]
        if grp is None:
            q_items = [(('qmm', g), 16) for g in range(10)]
        else:
            q_items = [(('qmm', g), 24) for g in range(5 * grp[1], 5 * grp[1] + 5)]
        do_exp = grp is None or grp[1] == 1
        wo_items = [(('wo', v), 24) for v in range(5)]
        qa, wa = cfg.get('q_at', 0), cfg.get('wo_at', 12)
        mx = list(qk_items)
        e_items = [(('qexpl',), 16)] if do_exp else []
        ins = sorted(((qa, 0, q_items), (cfg.get('e_at', 8), 1, e_items), (wa, 2, wo_items)), reverse=True)
        for at, _, items in ins:
            mx[at:at] = items
        tot = float(sum(w for _, w in mx))
        acc = 0
        for it, w in mx:
            acc += w
            p_ = start + (span - start) * acc / tot
            pos.append((p_, it))
            if it[0] == 'wo':
                pos.append((p_ - cfg.get('oahead', 0.03), ('ol', it[1])))
        if q and do_exp:
            pos.append((cfg.get('qexp', 0.6), ('qexps',)))
        if qk:
            pos.append((-1.0, ('bl',)))
        if next_bases:
            pos.append((cfg.get('bln', 0.7), ('bln',)))
        if sm:
            pos.append((-0.8, ('sml', 0)))
            pos.append((-0.7, ('sml', 1)))
            pos.append((cfg.get('sms', 0.6), ('sms', 0)))
            pos.append((cfg.get('sms', 0.6) + 0.01, ('sms', 1)))
        if wo:
            rows = [16 * b + r for r in range(16) for b in range(2 if wo_off else 3)]
            wl0, wl1 = cfg.get('wl0', 0.0), cfg.get('wl1', 0.2)
            for i, k in enumerate(rows):
                pos.append((wl0 + (wl1 - wl0) * i / len(rows), ('worow', k)))
            pos.append((wl1 + 1e-4, ('wof',)))
        on = dict(q=q, qk=qk, sm=sm, pv=pv, wo=wo)
        pos = [e for e in pos if on[stage_of[e[1][0]]]]
        pos.sort(key=lambda e: e[0])
        if guard is None:
            for _, it in pos:
                fn[it[0]](*it[1:])
        else:
            for stage in ('q', 'qk', 'sm', 'pv', 'wo'):
                items = [it for _, it in pos if stage_of[it[0]] == stage]

                def run(items=items):
                    for it in items:
                        fn[it[0]](*it[1:])
                guard(stage, run)
        return tmp.get('nb')


def _kernel(x_hbm, zs_hbm, k_hbm, v_hbm, wq_hbm, wo_hbm, w3_hbm, w4_hbm, o_ref,
            kb, vb, wqb, wob, wos, w3b, w4b, buf, eb, xb, x_ref, zs, sems, *, w_rows, n_rows):
    k32 = k_hbm.bitcast(jnp.uint32)
    v32 = v_hbm.bitcast(jnp.uint32)
    r0 = n_rows - w_rows

    def cp_k(j):
        return pltpu.make_async_copy(
            k32.at[pl.ds(2 * j, 2 * KVG), :, pl.ds(r0, w_rows), :], kb.at[pl.ds(2 * j, 2 * KVG)], sems.at[j])

    def cp_v(j):
        return pltpu.make_async_copy(
            v32.at[pl.ds(2 * j, 2 * KVG), :, pl.ds(r0, w_rows), :], vb.at[pl.ds(2 * j, 2 * KVG)], sems.at[NP + j])

    def cp_wo(j):
        return pltpu.make_async_copy(
            wo_hbm.at[pl.ds(2 * DH * j, 2 * DH), :], wos.at[j & 3], sems.at[2 * NP + j])

    cp_wq = pltpu.make_async_copy(wq_hbm.bitcast(jnp.uint32), wqb, sems.at[3 * NP])
    cp_w3 = pltpu.make_async_copy(w3_hbm, w3b, sems.at[3 * NP + 1])
    cw = F // W4_CHUNKS

    def cp_w4(c):
        return pltpu.make_async_copy(w4_hbm.at[pl.ds(cw * c, cw)], w4b.at[pl.ds(cw * c, cw)],
                                     sems.at[3 * NP + 4 + c])

    cp_x = pltpu.make_async_copy(x_hbm, x_ref, sems.at[3 * NP + 2])
    cp_z = pltpu.make_async_copy(zs_hbm, zs, sems.at[3 * NP + 3])

    def valid(j):
        return jnp.logical_and(j >= 0, j < NP)

    def clamp(j):
        return jnp.clip(j, 0, NP - 1)

    def start_group(t):
        for cp, j, g in ((cp_k, t, KVG), (cp_v, t - 2, KVG), (cp_wo, t - 3, 1)):
            if isinstance(j, int):
                if 0 <= j < NP and j % g == 0:
                    cp(j).start()
            else:
                @pl.when(jnp.logical_and(valid(j), (j & (g - 1)) == 0))
                def _(cp=cp, j=j):
                    cp(clamp(j) & -g).start()

    def wait_group(t):
        for cp, j, g in ((cp_k, t, KVG), (cp_v, t - 2, KVG), (cp_wo, t - 3, 1)):
            @pl.when(jnp.logical_and(valid(j), (j & (g - 1)) == 0))
            def _(cp=cp, j=j):
                cp(clamp(j) & -g).wait()

    cp_wq.start()
    cp_x.start()
    cp_z.start()
    for t in (0, 1):
        start_group(t)
    cp_z.wait()
    cp_x.wait()

    att = _Attn(kb, vb, wqb, wob, buf, zs, eb, xb)
    att.init_expander()

    def attention_streaming(x):
        att.set_x(x)
        att.zero_out()
        cp_wq.wait()

        def body(t, carry):
            wait_group(t)

            @pl.when(t >= 3)
            def _():
                j = t - 3
                for v in range(D // LANES):
                    wob[j, v] = pltpu.bitcast(wos[j & 3, :, pl.ds(LANES * v, LANES)], jnp.uint32)
            start_group(t + 3)

            @pl.when(t == NP - 1)
            def _():
                cp_w3.start()
                for c in range(W4_CHUNKS):
                    cp_w4(c).start()

            first = dict(q=-1, qk=0, sm=1, pv=2, wo=3)

            def guard(stage, run):
                pl.when(jnp.logical_and(t >= first[stage], t < first[stage] + NP))(run)
            att.step(t, guard=guard)
            return carry
        jax.lax.fori_loop(-1, NP + 3, body, 0)
        return x + att.read_out()

    def attention_resident(x):
        att.set_x(x)
        att.zero_out()
        att.step(-2, qk=False, sm=False, pv=False, wo=False, grp=(-1, 0))
        att.step(-1, qk=False, sm=False, pv=False, wo=False, grp=(-1, 1))
        nb = att.step(0, sm=False, pv=False, wo=False, grp=(0, 0), next_bases=True)
        att.step(1, pv=False, wo=False, grp=(0, 1), bases=nb)

        def body(b, carry):
            nb = att.step(2 * b, clamp_idx=True, grp=(b, 0), next_bases=True)
            att.step(2 * b + 1, clamp_idx=True, grp=(b, 1), bases=nb)
            return carry
        voff = bool(CFG.get('peel') and CFG.get('voff'))
        if CFG.get('peel'):
            jax.lax.fori_loop(1, NP // 2, body, 0)

            @pl.when(zs[0] == 0)
            def _():
                att.step(NP, q=False, qk=False, cfg=CFG.get('tail'), voff=voff)
                att.step(NP + 1, q=False, qk=False, sm=False, cfg=CFG.get('tail'), voff=voff, wo_off=voff)
        else:
            jax.lax.fori_loop(1, NP // 2 + 1, body, 0)
        att.step(NP + 2, q=False, qk=False, sm=False, pv=False, wo_off=voff)
        return x + att.read_out()

    def mixer(x, first):
        y = _ln(x)
        z = jnp.broadcast_to(_ln_centred(y), (16, D)).astype(jnp.bfloat16)
        if first:
            cp_w3.wait()
        h = jnp.dot(z, w3b[...], preferred_element_type=jnp.float32)
        h = jax.nn.gelu(h, approximate=True).astype(jnp.bfloat16)
        h2 = None
        for c in range(W4_CHUNKS):
            if first:
                cp_w4(c).wait()
            d = jnp.dot(h[:, cw * c:cw * (c + 1)], w4b[pl.ds(cw * c, cw), :], preferred_element_type=jnp.float32)[0:8]
            h2 = d if h2 is None else h2 + d
        return x + (y + h2[0:1])

    x = x_ref[...].astype(jnp.float32)
    x = attention_streaming(x)
    x = mixer(x, True)
    x = attention_resident(x)
    x = mixer(x, False)
    o_ref[...] = x.astype(o_ref.dtype)


def _tile_view(c):
    _, h, s, dh = c.shape
    return (c.reshape(h, s // LANES, LANES, dh // 8, 8)
            .transpose(0, 3, 1, 4, 2)
            .reshape(h, dh // 8, s // LANES * 8, LANES))


@jax.jit
def pallas_interleave_layers__sliding_block_cached__mixer_s_mlp__decode_kernel(
    A_x: jax.Array,
    A_k_cache: jax.Array,
    A_v_cache: jax.Array,
    A_wq: jax.Array,
    A_wo: jax.Array,
    B_x: jax.Array,
    B_w1: jax.Array,
    B_w2: jax.Array,
    B_w3: jax.Array,
    B_w4: jax.Array,
):
    del B_x, B_w1, B_w2
    s = A_k_cache.shape[2]
    w = min(4096, max(256, s // 4))
    w_rows = w // LANES * 4
    n_rows = s // LANES * 4
    kk = _tile_view(A_k_cache)
    vv = _tile_view(A_v_cache)
    wq_t = (A_wq.reshape(D // 8, 8, H * DH // LANES, LANES).transpose(0, 2, 1, 3)
            .reshape(D // 8, H * DH // LANES * 8, LANES))
    any_spec = pl.BlockSpec(memory_space=pl.ANY)
    out = pl.pallas_call(
        functools.partial(_kernel, w_rows=w_rows, n_rows=n_rows),
        out_shape=jax.ShapeDtypeStruct((1, D), A_x.dtype),
        in_specs=[any_spec] * 8,
        out_specs=pl.BlockSpec(memory_space=pltpu.VMEM),
        scratch_shapes=[
            pltpu.VMEM((H, 24, w_rows, LANES), jnp.uint32),
            pltpu.VMEM((H, 24, w_rows, LANES), jnp.uint32),
            pltpu.VMEM((D // 8, H * DH // LANES * 4, LANES), jnp.uint32),
            pltpu.VMEM((NP, D // LANES, DH, LANES), jnp.uint32),
            pltpu.VMEM((4, 2 * DH, D), jnp.bfloat16),
            pltpu.VMEM((D, F), jnp.bfloat16),
            pltpu.VMEM((F, D), jnp.bfloat16),
            pltpu.VMEM((R_END, LANES), jnp.float32),
            pltpu.VMEM((4, LANES // 2, LANES), jnp.uint32),
            pltpu.VMEM((10, 8, LANES), jnp.uint32),
            pltpu.VMEM((1, D), A_x.dtype),
            pltpu.SMEM((8,), jnp.int32),
            pltpu.SemaphoreType.DMA((3 * NP + 4 + W4_CHUNKS,)),
        ],
        compiler_params=pltpu.CompilerParams(vmem_limit_bytes=127 * 1024 * 1024,
                                             flags=CFG.get('flags')),
    )(A_x.reshape(1, D), jnp.zeros((8,), jnp.int32), kk, vv, wq_t, A_wo, B_w3, B_w4)
    return out.reshape(A_x.shape)
```
